```python
import jax
import jax.numpy as jnp

def _softmax(x, axis=-1):
    return jax.nn.softmax(x, axis=axis)
def _gelu(x):
    return jax.nn.gelu(x, approximate=True)
def _silu(x):
    return jax.nn.silu(x)
def _sigmoid(x):
    return jax.nn.sigmoid(x)
def _layernorm(x, axis=-1, eps=1e-5):
    m = jnp.mean(x, axis=axis, keepdims=True)
    v = jnp.var(x, axis=axis, keepdims=True)
    return (x - m) / jnp.sqrt(v + eps)
def _scatter_add(tgt, idx, src, axis=0):
    return tgt.at[idx].add(src)
def _segment_sum(src, seg, n):
    return jax.ops.segment_sum(src, seg, n)
class _Rng:
    def __init__(self, key):
        self._k = key
    def _next(self):
        self._k, sub = jax.random.split(self._k)
        return sub
    def normal(self, shape):
        return jax.random.normal(self._next(), shape, dtype=jnp.bfloat16)
    def randint(self, lo, hi, shape):
        return jax.random.randint(self._next(), shape, lo, hi, dtype=jnp.int32)
    def uniform(self, shape, lo=0.0, hi=1.0):
        return jax.random.uniform(self._next(), shape, jnp.bfloat16, lo, hi)
    def permutation(self, n):
        return jax.random.permutation(self._next(), n)


kernel_name = 'standalone__adm_resblock__diffusion'

def setup_inputs():
    _rng = _Rng(jax.random.key(int.from_bytes(__import__("os").urandom(4), "little")))
    _w = (lambda a: (lambda t: t.astype(jnp.bfloat16) if jnp.issubdtype(t.dtype, jnp.floating) else t)(jnp.asarray(a)))
    B, C, HW, E = 2, 512, 64, 1152
    sc = (9.0 * C) ** -0.5
    return {
        "x": _w((lambda *s: _rng.normal(s) * 0.05)(B, C, HW, HW)),
        "t_emb": _w((lambda *s: _rng.normal(s) * 0.05)(B, E)),
        "g1": _w(1.0 + 0.1 * (lambda *s: _rng.normal(s) * 0.05)(C)),
        "be1": _w(0.1 * (lambda *s: _rng.normal(s) * 0.05)(C)),
        "w1": _w((lambda *s: _rng.normal(s) * 0.05)(C, C, 3, 3) * sc),
        "w_emb": _w((lambda *s: _rng.normal(s) * 0.05)(E, C) * (E ** -0.5)),
        "g2": _w(1.0 + 0.1 * (lambda *s: _rng.normal(s) * 0.05)(C)),
        "be2": _w(0.1 * (lambda *s: _rng.normal(s) * 0.05)(C)),
        "w2": _w((lambda *s: _rng.normal(s) * 0.05)(C, C, 3, 3) * sc),
    }

def reference(x, t_emb, g1, be1, w1, w_emb, g2, be2, w2):
    B, C, H, W = x.shape
    G, eps = 4, 1e-5
    def gn(z, gamma, beta):
        zr = z.reshape(B, G, (C // G) * H * W)
        mu = zr.mean(-1).reshape(B, G, 1)
        var = ((zr - mu) ** 2).mean(-1).reshape(B, G, 1)
        zn = ((zr - mu) / jnp.sqrt(var + eps)).reshape(B, C, H, W)
        return zn * gamma.reshape(1, C, 1, 1) + beta.reshape(1, C, 1, 1)
    def conv3(z, w):
        zp = jnp.pad(z, ((0, 0), (0, 0), (1, 1), (1, 1)))
        taps = [jnp.einsum("bchw,oc->bohw", zp[:, :, i:i+H, j:j+W], w[:, :, i, j]) for i in range(3) for j in range(3)]
        out = taps[0]
        for t in taps[1:]:
            out = out + t
        return out
    h = conv3(_silu(gn(x, g1, be1)), w1)
    emb = _silu(t_emb) @ w_emb
    h = h + emb.reshape(B, C, 1, 1)
    h = conv3(_silu(gn(h, g2, be2)), w2)
    return x + h
```

```python
import functools
import numpy as np
import jax
import jax.numpy as jnp
from jax.experimental import pallas as pl
from jax.experimental.pallas import tpu as pltpu

B, C, H, W, EMB = 2, 512, 64, 64, 1152
NG, LG = 4, 128
TH = 4
NP, NQ = 6, 4
NPOS = NP * NQ
TW = W // 2
CT = 4
MC = CT * TW
RC = CT * TH
NCH = H // RC
EPS = 1e-5
F32 = jnp.float32
BF16 = jnp.bfloat16
U32 = jnp.uint32

PA, PB = 2.0 / 3.0, 1.5


def _g_matrix():
    pts = [0.0, PA, -PA, PB, -PB]
    g = []
    for i, p in enumerate(pts):
        den = 1.0
        for j, q in enumerate(pts):
            if j != i:
                den *= (p - q)
        g.append([1.0 / den, p / den, p * p / den])
    g.append([0.0, 0.0, 1.0])
    return g

GH = _g_matrix()


def _bt_h(d):
    a2, b2 = PA * PA, PB * PB
    d0, d1, d2, d3, d4, d5 = d
    p2 = b2 * d2
    aa = d4 - p2
    ra = PA * (d3 - b2 * d1)
    ab = d4 - a2 * d2
    rb = PB * (d3 - a2 * d1)
    t0 = (d0 + ab) - p2
    t5 = (d1 + d5) - (a2 + b2) * d3
    return [t0, aa + ra, aa - ra, ab + rb, ab - rb, t5]


def _at_h(m):
    m0, m1, m2, m3, m4, m5 = m
    sa, da = m1 + m2, m1 - m2
    sb, db = m3 + m4, m3 - m4
    y0 = (m0 + sa) + sb
    y1 = PA * da + PB * db
    y2 = (PA * PA) * sa + (PB * PB) * sb
    y3 = ((PA ** 3) * da + (PB ** 3) * db) + m5
    return [y0, y1, y2, y3]


def _unpack(w):
    lo = pltpu.unpack_elementwise(w, index=0, packed_dtype=BF16, unpacked_dtype=F32)
    hi = pltpu.unpack_elementwise(w, index=1, packed_dtype=BF16, unpacked_dtype=F32)
    return lo, hi


def _pack(lo, hi):
    return pltpu.pack_elementwise([lo, hi], packed_dtype=BF16)


def _gs(g):
    return slice(g * LG, (g + 1) * LG)


def make_kernel(cfg):
    def kernel(x_hbm, t_ref, g1_ref, be1_ref, w1_hbm, wemb_hbm, g2_ref, be2_ref, w2_hbm,
               out_hbm,
               xs, wraw, wembs, u_ref, src, v0, v1, m0, m1, shb, stats, embtab, gbt, sems):
        vbuf = (v0, v1)
        mbuf = (m0, m1)

        def x_stats(img, row0, nrows, slot):
            for g in range(NG):
                a1 = jnp.zeros((TW, LG), F32)
                a2 = jnp.zeros((TW, LG), F32)
                for j in range(nrows):
                    r = row0 + j
                    w = pltpu.bitcast(xs[img, r, :, _gs(g)], U32)
                    src[img, r, :, _gs(g)] = w
                    e, o = _unpack(w)
                    a1 = a1 + (e + o)
                    a2 = a2 + (e * e + o * o)
                stats[img, slot, 0, :, _gs(g)] = a1.reshape(4, 8, LG).sum(axis=0)
                stats[img, slot, 1, :, _gs(g)] = a2.reshape(4, 8, LG).sum(axis=0)

        def w_transform(conv, ob, nob):
            for cb in range(NG):
                we = [[None] * 3 for _ in range(3)]
                wo = [[None] * 3 for _ in range(3)]
                for i in range(3):
                    for j in range(3):
                        w = pltpu.bitcast(wraw[conv, i, j, pl.ds(2 * ob, 2 * nob), _gs(cb)], U32)
                        we[i][j], wo[i][j] = _unpack(w)
                res = []
                for par in (we, wo):
                    wq = []
                    for i in range(3):
                        s = par[i][0] + par[i][2]
                        wq.append([par[i][0], s + par[i][1], s - par[i][1], par[i][2]])
                    out = [[None] * NQ for _ in range(NP)]
                    for q in range(NQ):
                        sc = 0.5 if q in (1, 2) else 1.0
                        g0, g1, g2 = wq[0][q], wq[1][q], wq[2][q]
                        out[0][q] = (GH[0][0] * sc) * g0
                        for pp in (1, 3):
                            ev = (GH[pp][0] * sc) * g0 + (GH[pp][2] * sc) * g2
                            od = (GH[pp][1] * sc) * g1
                            out[pp][q] = ev + od
                            out[pp + 1][q] = ev - od
                        out[5][q] = g2 if sc == 1.0 else sc * g2
                    res.append(out)
                for p in range(NP):
                    for q in range(NQ):
                        u_ref[conv, p * NQ + q, pl.ds(ob, nob), _gs(cb)] = _pack(res[0][p][q], res[1][p][q])

        def gn_params(sidx, conv):
            s1 = stats[sidx, 0, 0] + stats[sidx, 1, 0] + stats[sidx, 2, 0] + stats[sidx, 3, 0]
            s2 = stats[sidx, 0, 1] + stats[sidx, 1, 1] + stats[sidx, 2, 1] + stats[sidx, 3, 1]
            s1 = jnp.sum(s1, axis=0, keepdims=True)
            s2 = jnp.sum(s2, axis=0, keepdims=True)
            e = embtab[sidx]
            n = float(H * W)
            t1 = s1 + n * e
            t2 = s2 + (2.0 * e) * s1 + (n * e) * e
            gam = gbt[conv, 0]
            bet = gbt[conv, 1]
            scs, shs = [], []
            inv = 1.0 / (H * W * LG)
            for g in range(NG):
                mean = jnp.sum(t1[:, _gs(g)], axis=1, keepdims=True) * inv
                ex2 = jnp.sum(t2[:, _gs(g)], axis=1, keepdims=True) * inv
                var = jnp.maximum(ex2 - mean * mean, 0.0)
                rstd = jax.lax.rsqrt(var + EPS)
                sc = gam[:, _gs(g)] * rstd
                sh = bet[:, _gs(g)] + (e[:, _gs(g)] - mean) * sc
                scs.append(0.5 * sc)
                shs.append(0.5 * sh)
            return scs, shs

        def stage_in(s, vdst, edge):
            sidx = s // 4
            chunk = s % 4
            scs, shs = gn_params(sidx, sidx // 2)
            r0 = chunk * RC - 1
            for g in range(NG):
                sc, sh = scs[g], shs[g]
                acts = []
                for j in range(RC + 2):
                    r = r0 + j
                    valid = None
                    if isinstance(r, int):
                        if r < 0 or r >= H:
                            z = jnp.zeros((TW, LG), F32)
                            acts.append((z, z))
                            continue
                    else:
                        if j == 0 and edge in ('top', 'both'):
                            valid = r >= 0
                            r = jnp.maximum(r, 0)
                        if j == RC + 1 and edge in ('bot', 'both'):
                            valid = r < H
                            r = jnp.minimum(r, H - 1)
                    w = src[sidx, r, :, _gs(g)]
                    pair = []
                    for z in _unpack(w):
                        hv = z * sc + sh
                        a = hv + hv * jnp.tanh(hv)
                        if valid is not None:
                            a = jnp.where(valid, a, 0.0)
                        pair.append(a)
                    acts.append(tuple(pair))
                for ty in range(CT):
                    rows = acts[ty * TH: ty * TH + NP]
                    te = _bt_h([rw[0] for rw in rows])
                    to = _bt_h([rw[1] for rw in rows])
                    for p in range(NP):
                        slot = (g * CT + ty) * NP + p
                        shb[slot, pl.ds(1, TW, stride=2), :] = te[p]
                        shb[slot, pl.ds(2, TW, stride=2), :] = to[p]
                        d0 = shb[slot, pl.ds(0, TW, stride=2), :]
                        d3 = shb[slot, pl.ds(3, TW, stride=2), :]
                        tq = [d0 - to[p], te[p] + to[p], to[p] - te[p], te[p] - d3]
                        for q in range(NQ):
                            vdst[p * NQ + q, pl.ds(ty * (TW // 2), TW // 2), _gs(g)] = pltpu.bitcast(
                                tq[q].astype(BF16), U32)

        def stage_mm(s, vsrc, mdst, p0=0, p1=NPOS):
            conv = s // 8
            for pos in range(p0, p1):
                v = pltpu.bitcast(vsrc[pos], BF16)
                u = pltpu.bitcast(u_ref[conv, pos], BF16)
                mdst[pos] = jax.lax.dot_general(v, u, (((1,), (1,)), ((), ())),
                                                preferred_element_type=F32)

        def stage_out(s, msrc, kind):
            img = (s // 4) % 2
            chunk = s % 4
            for g in range(NG):
                a1 = jnp.zeros((TW, LG), F32)
                a2 = jnp.zeros((TW, LG), F32)
                for ty in range(CT):
                    z0, z1 = [], []
                    for p in range(NP):
                        mm = [msrc[p * NQ + q, pl.ds(ty * TW, TW), _gs(g)] for q in range(NQ)]
                        z0.append((mm[0] + mm[1]) + mm[2])
                        z1.append((mm[1] - mm[2]) - mm[3])
                    ye = _at_h(z0)
                    yo = _at_h(z1)
                    for k in range(TH):
                        r = chunk * RC + ty * TH + k
                        if kind == 1:
                            a1 = a1 + (ye[k] + yo[k])
                            a2 = a2 + (ye[k] * ye[k] + yo[k] * yo[k])
                            src[2 + img, r, :, _gs(g)] = _pack(ye[k], yo[k])
                        else:
                            xe, xo = _unpack(src[img, r, :, _gs(g)])
                            xs[img, r, :, _gs(g)] = pltpu.bitcast(_pack(ye[k] + xe, yo[k] + xo), BF16)
                if kind == 1:
                    stats[2 + img, chunk, 0, :, _gs(g)] = a1.reshape(4, 8, LG).sum(axis=0)
                    stats[2 + img, chunk, 1, :, _gs(g)] = a2.reshape(4, 8, LG).sum(axis=0)

        def out_copy(s):
            img = (s // 4) % 2
            chunk = s % 4
            return pltpu.make_async_copy(xs.at[img, pl.ds(chunk * RC, RC)],
                                         out_hbm.at[img, pl.ds(chunk * RC, RC)],
                                         sems.at[8 + (s - 8)])

        cx0 = pltpu.make_async_copy(x_hbm.at[0], xs.at[0], sems.at[0])
        cw1 = pltpu.make_async_copy(w1_hbm, wraw.at[0], sems.at[1])
        cx1 = pltpu.make_async_copy(x_hbm.at[1], xs.at[1], sems.at[2])
        cw2 = pltpu.make_async_copy(w2_hbm, wraw.at[1], sems.at[3])
        cwe = pltpu.make_async_copy(wemb_hbm, wembs, sems.at[4])
        cx0.start(); cw1.start(); cx1.start(); cw2.start(); cwe.start()

        shb[...] = jnp.zeros(shb.shape, F32)
        gbt[0, 0] = g1_ref[...].astype(F32)
        gbt[0, 1] = be1_ref[...].astype(F32)
        gbt[1, 0] = g2_ref[...].astype(F32)
        gbt[1, 1] = be2_ref[...].astype(F32)

        cx0.wait()

        def xs_loop(img):
            def body(c, carry):
                x_stats(img, c * RC, RC, c)
                return carry
            jax.lax.fori_loop(0, NCH, body, 0)
        xs_loop(0)

        cw1.wait()

        def wt_loop(conv):
            def body(i, carry):
                w_transform(conv, pl.multiple_of(i * 32, 32), 32)
                return carry
            jax.lax.fori_loop(0, 8, body, 0)
        wt_loop(0)

        cwe.wait()
        t = t_ref[...].astype(F32)
        st = (t * jax.nn.sigmoid(t)).astype(BF16)
        emb = jnp.dot(st, wembs[...], preferred_element_type=F32)
        zero = jnp.zeros((1, C), F32)
        embtab[0] = zero
        embtab[1] = zero
        embtab[2] = emb[0:1]
        embtab[3] = emb[1:2]

        cx1.wait()
        xs_loop(1)
        cw2.wait()
        wt_loop(1)

        stage_in(0, v0, None)

        stage_in(1, v1, None)
        stage_mm(0, v0, m0)

        def loop_a(i, carry):
            s = 2 * i + 1
            stage_out(s - 1, m0, 1)
            stage_in(s + 1, v0, 'top')
            stage_mm(s, v1, m1)
            s = 2 * i + 2
            stage_out(s - 1, m1, 1)
            stage_in(s + 1, v1, 'bot')
            stage_mm(s, v0, m0)
            return carry
        jax.lax.fori_loop(0, 4, loop_a, 0)

        def loop_b(i, carry):
            s = 2 * i + 1
            stage_out(s - 1, m0, 2)
            stage_in(s + 1, v0, 'top')
            stage_mm(s, v1, m1)
            s = 2 * i + 2
            stage_out(s - 1, m1, 2)
            stage_in(s + 1, v1, 'bot')
            stage_mm(s, v0, m0)
            out_copy(s - 2).start()
            out_copy(s - 1).start()
            return carry
        jax.lax.fori_loop(4, 7, loop_b, 0)

        stage_out(14, m0, 2)
        stage_mm(15, v1, m1)
        out_copy(14).start()
        stage_out(15, m1, 2)
        out_copy(15).start()
        for s in range(8, 16):
            out_copy(s).wait()

    return kernel


_KERNEL = make_kernel({})


@jax.jit
def pallas_standalone__adm_resblock__diffusion_kernel(x, t_emb, g1, be1, w1, w_emb, g2, be2, w2):
    xh = jnp.transpose(x, (0, 2, 3, 1))
    w1t = jnp.transpose(w1, (2, 3, 0, 1))
    w2t = jnp.transpose(w2, (2, 3, 0, 1))
    vm = pl.BlockSpec(memory_space=pltpu.VMEM)
    hb = pl.BlockSpec(memory_space=pl.ANY)
    out = pl.pallas_call(
        _KERNEL,
        out_shape=jax.ShapeDtypeStruct((B, H, W, C), BF16),
        in_specs=[hb, vm, vm, vm, hb, hb, vm, vm, hb],
        out_specs=hb,
        scratch_shapes=[
            pltpu.VMEM((B, H, W, C), BF16),
            pltpu.VMEM((2, 3, 3, C, C), BF16),
            pltpu.VMEM((EMB, C), BF16),
            pltpu.VMEM((2, NPOS, C // 2, C), U32),
            pltpu.VMEM((4, H, TW, C), U32),
            pltpu.VMEM((NPOS, MC // 2, C), U32),
            pltpu.VMEM((NPOS, MC // 2, C), U32),
            pltpu.VMEM((NPOS, MC, C), F32),
            pltpu.VMEM((NPOS, MC, C), F32),
            pltpu.VMEM((NG * CT * NP, 72, LG), F32),
            pltpu.VMEM((4, NCH, 2, 8, C), F32),
            pltpu.VMEM((4, 1, C), F32),
            pltpu.VMEM((2, 2, 1, C), F32),
            pltpu.SemaphoreType.DMA((16,)),
        ],
        compiler_params=pltpu.CompilerParams(vmem_limit_bytes=120 * 2 ** 20),
    )(xh, t_emb, g1.reshape(1, C), be1.reshape(1, C), w1t, w_emb, g2.reshape(1, C), be2.reshape(1, C), w2t)
    return jnp.transpose(out, (0, 3, 1, 2))
```

```python
import functools
import numpy as np
import jax
import jax.numpy as jnp
from jax.experimental import pallas as pl
from jax.experimental.pallas import tpu as pltpu

B, C, H, W, EMB = 2, 512, 64, 64, 1152
NG, LG = 4, 128
TH = 4
NP, NQ = 6, 4
NPOS = NP * NQ
TW = W // 2
CT = 4
MC = CT * TW
RC = CT * TH
NCH = H // RC
EPS = 1e-5
F32 = jnp.float32
BF16 = jnp.bfloat16
U32 = jnp.uint32
NSL = 4
SHR = 40

PA, PB = 2.0 / 3.0, 1.5


def _g_matrix():
    pts = [0.0, PA, -PA, PB, -PB]
    g = []
    for i, p in enumerate(pts):
        den = 1.0
        for j, q in enumerate(pts):
            if j != i:
                den *= (p - q)
        g.append([1.0 / den, p / den, p * p / den])
    g.append([0.0, 0.0, 1.0])
    return g

GH = _g_matrix()


def _bt_h(d):
    a2, b2 = PA * PA, PB * PB
    d0, d1, d2, d3, d4, d5 = d
    p2 = b2 * d2
    aa = d4 - p2
    ra = PA * (d3 - b2 * d1)
    ab = d4 - a2 * d2
    rb = PB * (d3 - a2 * d1)
    t0 = (d0 + ab) - p2
    t5 = (d1 + d5) - (a2 + b2) * d3
    return [t0, aa + ra, aa - ra, ab + rb, ab - rb, t5]


def _at_h(m):
    m0, m1, m2, m3, m4, m5 = m
    sa, da = m1 + m2, m1 - m2
    sb, db = m3 + m4, m3 - m4
    y0 = (m0 + sa) + sb
    y1 = PA * da + PB * db
    y2 = (PA * PA) * sa + (PB * PB) * sb
    y3 = ((PA ** 3) * da + (PB ** 3) * db) + m5
    return [y0, y1, y2, y3]


def _unpack(w, idx):
    return pltpu.unpack_elementwise(w, index=idx, packed_dtype=BF16, unpacked_dtype=F32)


def _pack(lo, hi):
    return pltpu.pack_elementwise([lo, hi], packed_dtype=BF16)


def _gs(g):
    return slice(g * LG, (g + 1) * LG)


def _shr(s, k):
    return s >> k


def make_kernel(cfg):
    T_TARGET = cfg.get('T', 12000)

    def kernel(x_hbm, t_ref, g1_ref, be1_ref, w1_hbm, wemb_hbm, g2_ref, be2_ref, w2_hbm,
               out_hbm,
               xs, wraw, wembs, u_ref, src, v0, v1, m0, m1, shb, ast, stats, embtab, gbt, gnp, zsm, sems):
        vbuf = (v0, v1)
        mbuf = (m0, m1)

        def delay(tok_u32, n):
            t = pltpu.bitcast(tok_u32, F32)
            for _ in range(n):
                t = jnp.broadcast_to(jnp.sum(t, axis=1, keepdims=True), (8, LG))
            return t

        def run_chains(chains, paced=True):
            items = []
            for ci, ch in enumerate(chains):
                n = len(ch)
                nat = sum(c[1] for c in ch)
                nx_total = max(0, int(round((T_TARGET - nat) / 116.0)))
                for k, (fn, _) in enumerate(ch):
                    nx = ((k + 1) * nx_total) // n - (k * nx_total) // n
                    items.append(((k + 0.5) / n, ci, fn, nx))
            items.sort(key=lambda it: (it[0], it[1]))
            toks = [None] * len(chains)
            for _, ci, fn, nx in items:
                raw = fn(toks[ci])
                toks[ci] = delay(raw, nx) if paced else None

        def inj(x, tok):
            return x if tok is None else x + tok

        def x_stats(img, row0, nrows, slot):
            for g in range(NG):
                a1 = jnp.zeros((TW, LG), F32)
                a2 = jnp.zeros((TW, LG), F32)
                for j in range(nrows):
                    r = row0 + j
                    w = pltpu.bitcast(xs[img, r, :, _gs(g)], U32)
                    src[img, r, g] = w
                    e, o = _unpack(w, 0), _unpack(w, 1)
                    a1 = a1 + (e + o)
                    a2 = a2 + (e * e + o * o)
                stats[img, slot, 0, :, _gs(g)] = a1.reshape(4, 8, LG).sum(axis=0)
                stats[img, slot, 1, :, _gs(g)] = a2.reshape(4, 8, LG).sum(axis=0)

        def w_transform(conv, ob, nob):
            for cb in range(NG):
                we = [[None] * 3 for _ in range(3)]
                wo = [[None] * 3 for _ in range(3)]
                for i in range(3):
                    for j in range(3):
                        w = pltpu.bitcast(wraw[conv, i, j, pl.ds(2 * ob, 2 * nob), _gs(cb)], U32)
                        we[i][j], wo[i][j] = _unpack(w, 0), _unpack(w, 1)
                res = []
                for par in (we, wo):
                    wq = []
                    for i in range(3):
                        s = par[i][0] + par[i][2]
                        wq.append([par[i][0], s + par[i][1], s - par[i][1], par[i][2]])
                    out = [[None] * NQ for _ in range(NP)]
                    for q in range(NQ):
                        sc = 0.5 if q in (1, 2) else 1.0
                        g0, g1, g2 = wq[0][q], wq[1][q], wq[2][q]
                        out[0][q] = (GH[0][0] * sc) * g0
                        for pp in (1, 3):
                            ev = (GH[pp][0] * sc) * g0 + (GH[pp][2] * sc) * g2
                            od = (GH[pp][1] * sc) * g1
                            out[pp][q] = ev + od
                            out[pp + 1][q] = ev - od
                        out[5][q] = g2 if sc == 1.0 else sc * g2
                    res.append(out)
                for p in range(NP):
                    for q in range(NQ):
                        u_ref[conv, p * NQ + q, pl.ds(ob, nob), _gs(cb)] = _pack(res[0][p][q], res[1][p][q])

        def gn_params(sidx):
            conv = _shr(sidx, 1)
            s1 = stats[sidx, 0, 0] + stats[sidx, 1, 0] + stats[sidx, 2, 0] + stats[sidx, 3, 0]
            s2 = stats[sidx, 0, 1] + stats[sidx, 1, 1] + stats[sidx, 2, 1] + stats[sidx, 3, 1]
            s1 = jnp.sum(s1, axis=0, keepdims=True)
            s2 = jnp.sum(s2, axis=0, keepdims=True)
            e = embtab[sidx]
            n = float(H * W)
            t1 = s1 + n * e
            t2 = s2 + (2.0 * e) * s1 + (n * e) * e
            gam = gbt[conv, 0]
            bet = gbt[conv, 1]
            inv = 1.0 / (H * W * LG)
            for g in range(NG):
                mean = jnp.sum(t1[:, _gs(g)], axis=1, keepdims=True) * inv
                ex2 = jnp.sum(t2[:, _gs(g)], axis=1, keepdims=True) * inv
                var = jnp.maximum(ex2 - mean * mean, 0.0)
                rstd = jax.lax.rsqrt(var + EPS)
                sc = gam[:, _gs(g)] * rstd
                sh = bet[:, _gs(g)] + (e[:, _gs(g)] - mean) * sc
                gnp[sidx, 0, :, _gs(g)] = jnp.broadcast_to(0.5 * sc, (8, LG))
                gnp[sidx, 1, :, _gs(g)] = jnp.broadcast_to(0.5 * sh, (8, LG))

        def in_chain(s, vdst, edge):
            sidx = _shr(s, 2)
            chunk = s & 3
            r0 = chunk * RC - 1
            units = []

            def act_rows(g, ty, tpar, j, half, tok):
                sc = gnp[sidx, 0, :, _gs(g)]
                sh = gnp[sidx, 1, :, _gs(g)]
                sc = inj(sc, tok)
                pl_id = tpar * 2 + half
                rows = []
                for jr in range(NP):
                    lr = ty * TH + jr
                    if ty > 0 and jr < 2:
                        rows.append(ast[jr, pl_id, j])
                        continue
                    r = r0 + lr
                    valid = None
                    if isinstance(r, int):
                        if r < 0 or r >= H:
                            rows.append(jnp.zeros((8, LG), F32))
                            continue
                    else:
                        if lr == 0 and edge in ('top', 'both'):
                            valid = r >= 0
                            r = jnp.maximum(r, 0)
                        if lr == RC + 1 and edge in ('bot', 'both'):
                            valid = r < H
                            r = jnp.minimum(r, H - 1)
                    w = src[sidx, r, g, pl.ds(16 * j + tpar, 8, stride=2), :]
                    hv = _unpack(w, half) * sc + sh
                    a = hv + hv * jnp.tanh(hv)
                    if valid is not None:
                        a = jnp.where(valid, a, 0.0)
                    rows.append(a)
                if ty < CT - 1:
                    ast[0, pl_id, j] = rows[4]
                    ast[1, pl_id, j] = rows[5]
                return _bt_h(rows)

            cnt = 0
            for g in range(NG):
                for ty in range(CT):
                    sl = (cnt % NSL) * NP
                    cnt += 1

                    def u_shift(tok, g=g, ty=ty, sl=sl, which=0):
                        for j in range(2):
                            t = act_rows(g, ty, which, j, which, tok if j == 0 else None)
                            for p in range(NP):
                                shb[sl + p, pl.ds(1 + which + 16 * j, 8, stride=2), :] = t[p]
                        return pltpu.bitcast(shb[zsm[2], 0:8, :], U32)

                    hold = {}

                    def u_h(tok, g=g, ty=ty, j=0, hold=hold):
                        hold['oe'] = act_rows(g, ty, 0, j, 1, tok)
                        hold['eo'] = act_rows(g, ty, 1, j, 0, None)
                        return None

                    def u_w(tok, g=g, ty=ty, sl=sl, j=0, hold=hold, ps=range(NP)):
                        for p in ps:
                            ee = shb[sl + p, pl.ds(1 + 16 * j, 8, stride=2), :]
                            ee1 = shb[sl + p, pl.ds(3 + 16 * j, 8, stride=2), :]
                            oo = shb[sl + p, pl.ds(2 + 16 * j, 8, stride=2), :]
                            oo1 = shb[sl + p, pl.ds(16 * j, 8, stride=2), :]
                            oe, eo = hold['oe'][p], hold['eo'][p]
                            if p == ps[0]:
                                oe = inj(oe, tok)
                            tev = [oo1 - oe, ee + oe, oe - ee, ee - eo]
                            tod = [oe - oo, eo + oo, oo - eo, eo - ee1]
                            for q in range(NQ):
                                vdst[p * NQ + q, pl.ds(ty * 16 + 8 * j, 8), _gs(g)] = _pack(tev[q], tod[q])
                        return vdst[zsm[0], 0:8, 0:LG]

                    units.append((functools.partial(u_shift, which=0), 30))
                    units.append((functools.partial(u_shift, which=1), 30))
                    for j in range(2):
                        def u_hw(tok, j=j, u_h=u_h, u_w=u_w):
                            u_h(tok, j=j)
                            return u_w(None, j=j)
                        units.append((u_hw, 40))
            return units

        def out_chain(s, msrc, kind):
            img = _shr(s, 2) & 1
            chunk = s & 3
            units = []
            for g in range(NG):
                acc = [jnp.zeros((8, LG), F32), jnp.zeros((8, LG), F32)]
                for ty in range(CT):
                    for jj in range(4):
                        def unit(tok, g=g, ty=ty, jj=jj, acc=acc):
                            z0, z1 = [], []
                            for p in range(NP):
                                mm = [msrc[p * NQ + q, pl.ds(ty * TW + 8 * jj, 8), _gs(g)] for q in range(NQ)]
                                m1_ = inj(mm[1], tok) if p == 0 else mm[1]
                                z0.append((mm[0] + m1_) + mm[2])
                                z1.append((m1_ - mm[2]) - mm[3])
                            ye = _at_h(z0)
                            yo = _at_h(z1)
                            for k in range(TH):
                                r = chunk * RC + ty * TH + k
                                if kind == 1:
                                    acc[0] = acc[0] + (ye[k] + yo[k])
                                    acc[1] = acc[1] + (ye[k] * ye[k] + yo[k] * yo[k])
                                    src[2 + img, r, g, pl.ds(8 * jj, 8), :] = _pack(ye[k], yo[k])
                                else:
                                    xw = src[img, r, g, pl.ds(8 * jj, 8), :]
                                    xs[img, r, pl.ds(16 * jj, 16), _gs(g)] = pltpu.bitcast(
                                        _pack(ye[k] + _unpack(xw, 0), yo[k] + _unpack(xw, 1)), BF16)
                            if kind == 1 and ty == CT - 1 and jj == 3:
                                stats[2 + img, chunk, 0, :, _gs(g)] = acc[0]
                                stats[2 + img, chunk, 1, :, _gs(g)] = acc[1]
                            if kind == 1:
                                return src[0, zsm[1], 0, 0:8, :]
                            return pltpu.bitcast(xs[0, zsm[1], 0:16, 0:LG], U32)
                        units.append((unit, 26))
            return units

        def stage_mm(s, vsrc, mdst, p0=0, p1=NPOS):
            conv = _shr(s, 3)
            for pos in range(p0, p1):
                v = pltpu.bitcast(vsrc[pos], BF16)
                u = pltpu.bitcast(u_ref[conv, pos], BF16)
                mdst[pos] = jax.lax.dot_general(v, u, (((1,), (1,)), ((), ())),
                                                preferred_element_type=F32)

        def out_copy(s):
            img = _shr(s, 2) & 1
            chunk = s & 3
            return pltpu.make_async_copy(xs.at[img, pl.ds(chunk * RC, RC)],
                                         out_hbm.at[img, pl.ds(chunk * RC, RC)],
                                         sems.at[8 + (s - 8)])

        cx0 = pltpu.make_async_copy(x_hbm.at[0], xs.at[0, pl.ds(0, H)], sems.at[0])
        cw1 = pltpu.make_async_copy(w1_hbm, wraw.at[0], sems.at[1])
        cx1 = pltpu.make_async_copy(x_hbm.at[1], xs.at[1, pl.ds(0, H)], sems.at[2])
        cw2 = pltpu.make_async_copy(w2_hbm, wraw.at[1], sems.at[3])
        cwe = pltpu.make_async_copy(wemb_hbm, wembs, sems.at[4])
        cx0.start(); cw1.start(); cx1.start(); cw2.start(); cwe.start()

        shb[...] = jnp.zeros(shb.shape, F32)
        zsm[0] = NPOS
        zsm[1] = H
        zsm[2] = NSL * NP
        v0[NPOS] = jnp.zeros((MC // 2, C), U32)
        v1[NPOS] = jnp.zeros((MC // 2, C), U32)
        src[0, H] = jnp.zeros((NG, TW, LG), U32)
        xs[0, H] = jnp.zeros((W, C), BF16)
        gbt[0, 0] = g1_ref[...].astype(F32)
        gbt[0, 1] = be1_ref[...].astype(F32)
        gbt[1, 0] = g2_ref[...].astype(F32)
        gbt[1, 1] = be2_ref[...].astype(F32)

        cx0.wait()

        def xs_loop(img):
            def body(c, carry):
                x_stats(img, c * RC, RC, c)
                return carry
            jax.lax.fori_loop(0, NCH, body, 0)
        xs_loop(0)

        cw1.wait()

        def wt_loop(conv):
            def body(i, carry):
                w_transform(conv, pl.multiple_of(i * 32, 32), 32)
                return carry
            jax.lax.fori_loop(0, 8, body, 0)
        wt_loop(0)

        cwe.wait()
        t = t_ref[...].astype(F32)
        st = (t * jax.nn.sigmoid(t)).astype(BF16)
        emb = jnp.dot(st, wembs[...], preferred_element_type=F32)
        zero = jnp.zeros((1, C), F32)
        embtab[0] = zero
        embtab[1] = zero
        embtab[2] = emb[0:1]
        embtab[3] = emb[1:2]

        cx1.wait()
        xs_loop(1)
        cw2.wait()
        wt_loop(1)
        gn_params(0)
        gn_params(1)

        run_chains([in_chain(0, v0, None)], paced=False)

        run_chains([in_chain(1, v1, None)])
        stage_mm(0, v0, m0)

        def step(s, kind, par):
            cur, nxt = par, 1 - par
            run_chains([out_chain(s - 1, mbuf[nxt], kind),
                        in_chain(s + 1, vbuf[nxt], 'top' if par == 1 else 'bot')])
            stage_mm(s, vbuf[cur], mbuf[cur])
            gn_params(jnp.minimum(_shr(s + 2, 2), 3))

        def loop_a(s, carry):
            jax.lax.cond((s & 1) == 0, lambda: step(s, 1, 0), lambda: step(s, 1, 1))
            return carry
        jax.lax.fori_loop(1, 9, loop_a, 0)

        def loop_b(s, carry):
            jax.lax.cond((s & 1) == 0, lambda: step(s, 2, 0), lambda: step(s, 2, 1))
            out_copy(s - 1).start()
            return carry
        jax.lax.fori_loop(9, 15, loop_b, 0)

        run_chains([out_chain(14, m0, 2)])
        stage_mm(15, v1, m1)
        out_copy(14).start()
        run_chains([out_chain(15, m1, 2)], paced=False)
        out_copy(15).start()
        for s in range(8, 16):
            out_copy(s).wait()

    return kernel


_KERNEL = make_kernel({'T': 12000})


@jax.jit
def pallas_standalone__adm_resblock__diffusion_kernel(x, t_emb, g1, be1, w1, w_emb, g2, be2, w2):
    xh = jnp.transpose(x, (0, 2, 3, 1))
    w1t = jnp.transpose(w1, (2, 3, 0, 1))
    w2t = jnp.transpose(w2, (2, 3, 0, 1))
    vm = pl.BlockSpec(memory_space=pltpu.VMEM)
    hb = pl.BlockSpec(memory_space=pl.ANY)
    out = pl.pallas_call(
        _KERNEL,
        out_shape=jax.ShapeDtypeStruct((B, H, W, C), BF16),
        in_specs=[hb, vm, vm, vm, hb, hb, vm, vm, hb],
        out_specs=hb,
        scratch_shapes=[
            pltpu.VMEM((B, H + 1, W, C), BF16),
            pltpu.VMEM((2, 3, 3, C, C), BF16),
            pltpu.VMEM((EMB, C), BF16),
            pltpu.VMEM((2, NPOS, C // 2, C), U32),
            pltpu.VMEM((4, H + 1, NG, TW, LG), U32),
            pltpu.VMEM((NPOS + 1, MC // 2, C), U32),
            pltpu.VMEM((NPOS + 1, MC // 2, C), U32),
            pltpu.VMEM((NPOS, MC, C), F32),
            pltpu.VMEM((NPOS, MC, C), F32),
            pltpu.VMEM((NSL * NP + 1, SHR, LG), F32),
            pltpu.VMEM((2, 4, 2, 8, LG), F32),
            pltpu.VMEM((4, NCH, 2, 8, C), F32),
            pltpu.VMEM((4, 1, C), F32),
            pltpu.VMEM((2, 2, 1, C), F32),
            pltpu.VMEM((4, 2, 8, C), F32),
            pltpu.SMEM((4,), jnp.int32),
            pltpu.SemaphoreType.DMA((16,)),
        ],
        compiler_params=pltpu.CompilerParams(vmem_limit_bytes=120 * 2 ** 20),
    )(xh, t_emb, g1.reshape(1, C), be1.reshape(1, C), w1t, w_emb, g2.reshape(1, C), be2.reshape(1, C), w2t)
    return jnp.transpose(out, (0, 3, 1, 2))
```

```python
import functools
import numpy as np
import jax
import jax.numpy as jnp
from jax.experimental import pallas as pl
from jax.experimental.pallas import tpu as pltpu

B, C, H, W, EMB = 2, 512, 64, 64, 1152
NG, LG = 4, 128
TH = 4
NP, NQ = 6, 4
NPOS = NP * NQ
TW = W // 2
CT = 4
MC = CT * TW
RC = CT * TH
NCH = H // RC
EPS = 1e-5
F32 = jnp.float32
BF16 = jnp.bfloat16
U32 = jnp.uint32
NSL = 4
SHR = 40

PA, PB = 2.0 / 3.0, 1.5


def _g_matrix():
    pts = [0.0, PA, -PA, PB, -PB]
    g = []
    for i, p in enumerate(pts):
        den = 1.0
        for j, q in enumerate(pts):
            if j != i:
                den *= (p - q)
        g.append([1.0 / den, p / den, p * p / den])
    g.append([0.0, 0.0, 1.0])
    return g

GH = _g_matrix()


def _bt_h(d):
    a2, b2 = PA * PA, PB * PB
    d0, d1, d2, d3, d4, d5 = d
    p2 = b2 * d2
    aa = d4 - p2
    ra = PA * (d3 - b2 * d1)
    ab = d4 - a2 * d2
    rb = PB * (d3 - a2 * d1)
    t0 = (d0 + ab) - p2
    t5 = (d1 + d5) - (a2 + b2) * d3
    return [t0, aa + ra, aa - ra, ab + rb, ab - rb, t5]


def _at_h(m):
    m0, m1, m2, m3, m4, m5 = m
    sa, da = m1 + m2, m1 - m2
    sb, db = m3 + m4, m3 - m4
    y0 = (m0 + sa) + sb
    y1 = PA * da + PB * db
    y2 = (PA * PA) * sa + (PB * PB) * sb
    y3 = ((PA ** 3) * da + (PB ** 3) * db) + m5
    return [y0, y1, y2, y3]


def _unpack(w, idx):
    return pltpu.unpack_elementwise(w, index=idx, packed_dtype=BF16, unpacked_dtype=F32)


def _pack(lo, hi):
    return pltpu.pack_elementwise([lo, hi], packed_dtype=BF16)


def _gs(g):
    return slice(g * LG, (g + 1) * LG)


def _shr(s, k):
    return s >> k


def make_kernel(cfg):
    T_TARGET = cfg.get('T', 12000)

    def kernel(x_hbm, t_ref, g1_ref, be1_ref, w1_hbm, wemb_hbm, g2_ref, be2_ref, w2_hbm,
               out_hbm,
               wraw, wembs, u_ref, src, v0, v1, m0, m1, shb, ast, stats, embtab, gbt, gnp, xres, zvr, dum, zsm, sems):
        vbuf = (v0, v1)
        mbuf = (m0, m1)
        xb = x_hbm.bitcast(U32)
        ob_ = out_hbm.bitcast(U32)
        w1b = w1_hbm.bitcast(U32)
        w2b = w2_hbm.bitcast(U32)

        def delay(tok_u32, cyc):
            t = pltpu.bitcast(tok_u32, F32)
            n, rem = divmod(cyc, 116)
            if not cfg.get('fine', 1):
                rem = 0
            for _ in range(n):
                t = jnp.broadcast_to(jnp.sum(t, axis=1, keepdims=True), (8, LG))
            for _ in range(rem // cfg.get('eup', 8)):
                t = jnp.tanh(t)
            return t

        def run_chains(chains, paced=True):
            if cfg.get('merge', 0) and len(chains) > 1:
                tagged = []
                for ci, ch in enumerate(chains):
                    for k, it in enumerate(ch):
                        tagged.append(((k + 0.5) / len(ch), ci, it))
                tagged.sort(key=lambda t: (t[0], t[1]))
                chains = [[t[2] for t in tagged]]
            items = []
            for ci, ch in enumerate(chains):
                n = len(ch)
                nat = sum(c[1] for c in ch)
                slack = max(0, T_TARGET - nat)
                cum = 0
                if cfg.get('fine', 1):
                    per = T_TARGET / n
                    acc_t = 0.0
                    for k, (fn, lat) in enumerate(ch):
                        d = max(0, int(per - lat))
                        items.append(((k + 0.5) / n, ci, fn, d))
                else:
                    nx_total = int(round(slack / 116.0))
                    for k, (fn, _) in enumerate(ch):
                        nx = ((k + 1) * nx_total) // n - (k * nx_total) // n
                        items.append(((k + 0.5) / n, ci, fn, nx * 116))
            items.sort(key=lambda it: (it[0], it[1]))
            toks = [None] * len(chains)
            for _, ci, fn, nx in items:
                raw = fn(toks[ci])
                toks[ci] = delay(raw, nx) if paced else None
            if paced and cfg.get('tail', 0):
                for ci in range(len(chains)):
                    t = toks[ci]
                    for _ in range(cfg['tail'] // 116):
                        t = jnp.broadcast_to(jnp.sum(t, axis=1, keepdims=True), (8, LG))
                    dum[ci] = t

        L_S, L_H, L_W = cfg.get('L_S', 30), cfg.get('L_H', 30), cfg.get('L_W', 16)
        L_A, L_C = cfg.get('L_A', 20), cfg.get('L_C', 22)

        def anchor(vals):
            b = [pltpu.bitcast(v, U32) for v in vals]
            while len(b) > 1:
                b = [b[i] | b[i + 1] if i + 1 < len(b) else b[i] for i in range(0, len(b), 2)]
            return b[0] & zvr[...]

        def inj(x, tok):
            return x if tok is None else x + tok

        def x_stats(img, row0, nrows, slot):
            for g in range(NG):
                a1 = jnp.zeros((TW, LG), F32)
                a2 = jnp.zeros((TW, LG), F32)
                for j in range(nrows):
                    w = src[img, row0 + j, g]
                    e, o = _unpack(w, 0), _unpack(w, 1)
                    a1 = a1 + (e + o)
                    a2 = a2 + (e * e + o * o)
                stats[img, slot, 0, :, _gs(g)] = a1.reshape(4, 8, LG).sum(axis=0)
                stats[img, slot, 1, :, _gs(g)] = a2.reshape(4, 8, LG).sum(axis=0)

        def w_unit(conv, udst, ob, cb, tok=None):
            raw = [[[None] * 3 for _ in range(3)] for _ in range(2)]
            for i in range(3):
                for j in range(3):
                    w = wraw[conv, i, j, pl.ds(ob, 8), _gs(cb)]
                    raw[0][i][j], raw[1][i][j] = _unpack(w, 0), _unpack(w, 1)
            raw[0][0][0] = inj(raw[0][0][0], tok)
            sm = [[raw[par][i][0] + raw[par][i][2] for i in range(3)] for par in range(2)]
            for q in range(NQ):
                sc = 0.5 if q in (1, 2) else 1.0
                res = []
                for par in range(2):
                    r = raw[par]
                    if q == 0:
                        gq = [r[i][0] for i in range(3)]
                    elif q == 1:
                        gq = [sm[par][i] + r[i][1] for i in range(3)]
                    elif q == 2:
                        gq = [sm[par][i] - r[i][1] for i in range(3)]
                    else:
                        gq = [r[i][2] for i in range(3)]
                    g0, g1, g2 = gq
                    out = [None] * NP
                    out[0] = (GH[0][0] * sc) * g0
                    for pp in (1, 3):
                        ev = (GH[pp][0] * sc) * g0 + (GH[pp][2] * sc) * g2
                        od = (GH[pp][1] * sc) * g1
                        out[pp] = ev + od
                        out[pp + 1] = ev - od
                    out[5] = g2 if sc == 1.0 else sc * g2
                    res.append(out)
                for p in range(NP):
                    udst[p * NQ + q, pl.ds(ob, 8), _gs(cb)] = _pack(res[0][p], res[1][p])

        def emb_stage():
            t = t_ref[...].astype(F32)
            st = (t * jax.nn.sigmoid(t)).astype(BF16)
            emb = jnp.dot(st, wembs[...], preferred_element_type=F32)
            embtab[2] = emb[0:1]
            embtab[3] = emb[1:2]

        def gn_params(sidx):
            conv = _shr(sidx, 1)
            s1 = stats[sidx, 0, 0] + stats[sidx, 1, 0] + stats[sidx, 2, 0] + stats[sidx, 3, 0]
            s2 = stats[sidx, 0, 1] + stats[sidx, 1, 1] + stats[sidx, 2, 1] + stats[sidx, 3, 1]
            s1 = jnp.sum(s1, axis=0, keepdims=True)
            s2 = jnp.sum(s2, axis=0, keepdims=True)
            e = embtab[sidx]
            n = float(H * W)
            t1 = s1 + n * e
            t2 = s2 + (2.0 * e) * s1 + (n * e) * e
            gam = gbt[conv, 0]
            bet = gbt[conv, 1]
            inv = 1.0 / (H * W * LG)
            for g in range(NG):
                mean = jnp.sum(t1[:, _gs(g)], axis=1, keepdims=True) * inv
                ex2 = jnp.sum(t2[:, _gs(g)], axis=1, keepdims=True) * inv
                var = jnp.maximum(ex2 - mean * mean, 0.0)
                rstd = jax.lax.rsqrt(var + EPS)
                sc = gam[:, _gs(g)] * rstd
                sh = bet[:, _gs(g)] + (e[:, _gs(g)] - mean) * sc
                gnp[sidx, 0, :, _gs(g)] = jnp.broadcast_to(0.5 * sc, (8, LG))
                gnp[sidx, 1, :, _gs(g)] = jnp.broadcast_to(0.5 * sh, (8, LG))

        def in_chain(s, vdst, edge):
            sidx = _shr(s, 2)
            chunk = s & 3
            r0 = chunk * RC - 1
            units = []

            def act_rows(g, ty, tpar, j, half, tok):
                sc = gnp[sidx, 0, :, _gs(g)]
                sh = gnp[sidx, 1, :, _gs(g)]
                sc = inj(sc, tok)
                pl_id = tpar * 2 + half
                rows = []
                for jr in range(NP):
                    lr = ty * TH + jr
                    if ty > 0 and jr < 2:
                        rows.append(ast[jr, pl_id, j])
                        continue
                    r = r0 + lr
                    valid = None
                    if isinstance(r, int):
                        if r < 0 or r >= H:
                            rows.append(jnp.zeros((8, LG), F32))
                            continue
                    else:
                        if lr == 0 and edge in ('top', 'both'):
                            valid = r >= 0
                            r = jnp.maximum(r, 0)
                        if lr == RC + 1 and edge in ('bot', 'both'):
                            valid = r < H
                            r = jnp.minimum(r, H - 1)
                    if cfg.get('e_src'):
                        w = src[sidx, r, g, pl.ds(16 * j + 8 * tpar, 8), :]
                    else:
                        w = src[sidx, r, g, pl.ds(16 * j + tpar, 8, stride=2), :]
                    hv = _unpack(w, half) * sc + sh
                    a = hv + hv * (hv * hv if cfg.get('e_tanh') else jnp.tanh(hv))
                    if valid is not None:
                        a = jnp.where(valid, a, 0.0)
                    rows.append(a)
                if ty < CT - 1:
                    ast[0, pl_id, j] = rows[4]
                    ast[1, pl_id, j] = rows[5]
                return _bt_h(rows)

            cnt = 0
            for g in range(NG):
                for ty in range(CT):
                    sl = (cnt % NSL) * NP
                    cnt += 1

                    def u_shift(tok, g=g, ty=ty, sl=sl, which=0, js=(0, 1)):
                        for j in js:
                            t = act_rows(g, ty, which, j, which, tok if j == js[0] else None)
                            for p in range(NP):
                                if cfg.get('e_shb'):
                                    shb[sl + p, pl.ds(16 * which + 8 * j, 8), :] = t[p]
                                else:
                                    shb[sl + p, pl.ds(1 + which + 16 * j, 8, stride=2), :] = t[p]
                        return pltpu.bitcast(shb[zsm[2], 0:8, :], U32)

                    hold = {}

                    def u_h(tok, g=g, ty=ty, j=0, hold=hold):
                        hold['oe'] = act_rows(g, ty, 0, j, 1, tok)
                        hold['eo'] = act_rows(g, ty, 1, j, 0, None)
                        return None

                    def u_w(tok, g=g, ty=ty, sl=sl, j=0, hold=hold, ps=range(NP)):
                        for p in ps:
                            if cfg.get('e_shb'):
                                ee = shb[sl + p, pl.ds(8 * j, 8), :]
                                ee1 = shb[sl + p, pl.ds(8 + 8 * j, 8), :]
                                oo = shb[sl + p, pl.ds(16 + 8 * j, 8), :]
                                oo1 = shb[sl + p, pl.ds(24 + 8 * j, 8), :]
                            else:
                                ee = shb[sl + p, pl.ds(1 + 16 * j, 8, stride=2), :]
                                ee1 = shb[sl + p, pl.ds(3 + 16 * j, 8, stride=2), :]
                                oo = shb[sl + p, pl.ds(2 + 16 * j, 8, stride=2), :]
                                oo1 = shb[sl + p, pl.ds(16 * j, 8, stride=2), :]
                            oe, eo = hold['oe'][p], hold['eo'][p]
                            if p == ps[0]:
                                oe = inj(oe, tok)
                            tev = [oo1 - oe, ee + oe, oe - ee, ee - eo]
                            tod = [oe - oo, eo + oo, oo - eo, eo - ee1]
                            for q in range(NQ):
                                pk = _pack(tev[q], tod[q])
                                vdst[p * NQ + q, pl.ds(ty * 16 + 8 * j, 8), _gs(g)] = pk
                        if cfg.get('tokv'):
                            return pk & zvr[...]
                        return vdst[zsm[0], 0:8, 0:LG]

                    def u_h1(tok, g=g, ty=ty, j=0, hold=hold, key='oe'):
                        tpar, half = (0, 1) if key == 'oe' else (1, 0)
                        t = act_rows(g, ty, tpar, j, half, tok)
                        hold[key] = t
                        return anchor(t)

                    if cfg.get('ssplit', 1):
                        for which in range(2):
                            for j in range(2):
                                units.append((functools.partial(u_shift, which=which, js=(j,)), L_S))
                    else:
                        units.append((functools.partial(u_shift, which=0), 30))
                        units.append((functools.partial(u_shift, which=1), 30))
                    nsplit = cfg.get('wsplit', 3)
                    pg = [list(range(NP))[i * NP // nsplit:(i + 1) * NP // nsplit] for i in range(nsplit)]
                    for j in range(2):
                        if cfg.get('hsplit', 1):
                            units.append((functools.partial(u_h1, j=j, key='oe'), L_H))
                            units.append((functools.partial(u_h1, j=j, key='eo'), L_H))
                            for ps in pg:
                                units.append((functools.partial(u_w, j=j, ps=ps), L_W))
                        else:
                            def u_hw(tok, j=j, u_h=u_h, u_w=u_w):
                                u_h(tok, j=j)
                                return u_w(None, j=j, ps=pg[0])
                            units.append((u_hw, 40))
                            for ps in pg[1:]:
                                units.append((functools.partial(u_w, j=j, ps=ps), 14))
            return units

        def out_chain(s, msrc):
            img = _shr(s, 2) & 1
            chunk = s & 3
            if isinstance(s, int):
                kind2 = s >= 8
                dslot = (4 if kind2 else 2) + img
                sslot = 4 if kind2 else 2 + img
                rslot = img if kind2 else 0
            else:
                kind2 = s >= 8
                dslot = jnp.where(kind2, 4, 2) + img
                sslot = jnp.where(kind2, 4, 2 + img)
                rslot = jnp.where(kind2, img, 0)
            units = []
            for g in range(NG):
                acc = [jnp.zeros((8, LG), F32), jnp.zeros((8, LG), F32)]
                for ty in range(CT):
                    for jj in range(4):
                        hold = {}

                        def o_half(tok, g=g, ty=ty, jj=jj, hold=hold, par=0):
                            z = []
                            for p in range(NP):
                                qs = (0, 1, 2) if par == 0 else (1, 2, 3)
                                mm = [msrc[p * NQ + q, pl.ds(ty * TW + 8 * jj, 8), _gs(g)] for q in qs]
                                if p == 1:
                                    mm[0] = inj(mm[0], tok)
                                z.append((mm[0] + mm[1]) + mm[2] if par == 0 else (mm[0] - mm[1]) - mm[2])
                            y = _at_h(z)
                            hold[par] = y
                            return anchor(y)

                        def o_both(tok, g=g, ty=ty, jj=jj, hold=hold):
                            z0, z1 = [], []
                            for p in range(NP):
                                mm = [msrc[p * NQ + q, pl.ds(ty * TW + 8 * jj, 8), _gs(g)] for q in range(NQ)]
                                m1_ = inj(mm[1], tok) if p == 1 else mm[1]
                                z0.append((mm[0] + m1_) + mm[2])
                                z1.append((m1_ - mm[2]) - mm[3])
                            hold[0] = _at_h(z0)
                            hold[1] = _at_h(z1)

                        def o_fin(tok, g=g, ty=ty, jj=jj, acc=acc, hold=hold):
                            ye, yo = hold[0], hold[1]
                            xw = []
                            for k in range(TH):
                                r = chunk * RC + ty * TH + k
                                if isinstance(s, int):
                                    rr = r if kind2 else H
                                else:
                                    rr = jnp.where(kind2, r, H)
                                xw.append(src[rslot, rr, g, pl.ds(8 * jj, 8), :])
                            if tok is not None:
                                ye = [ye[0] + tok] + list(ye[1:])
                            for k in range(TH):
                                r = chunk * RC + ty * TH + k
                                if not (isinstance(s, int) and kind2):
                                    acc[0] = acc[0] + (ye[k] + yo[k])
                                    acc[1] = acc[1] + (ye[k] * ye[k] + yo[k] * yo[k])
                                pk = _pack(ye[k] + _unpack(xw[k], 0), yo[k] + _unpack(xw[k], 1))
                                src[dslot, r, g, pl.ds(8 * jj, 8), :] = pk
                            if ty == CT - 1 and jj == 3 and not (isinstance(s, int) and kind2):
                                stats[sslot, chunk, 0, :, _gs(g)] = acc[0]
                                stats[sslot, chunk, 1, :, _gs(g)] = acc[1]
                            tk = src[0, zsm[1], 0, 0:8, :]
                            if not (isinstance(s, int) and kind2):
                                tk = tk | ((pltpu.bitcast(acc[0], U32) | pltpu.bitcast(acc[1], U32)) & zvr[...])
                            return tk

                        osp = cfg.get('osplit', 3)
                        if osp == 3:
                            units.append((functools.partial(o_half, par=0), L_A))
                            units.append((functools.partial(o_half, par=1), L_A))
                            units.append((o_fin, L_C))
                        elif osp == 2:
                            def o_ab(tok, o_both=o_both, hold=hold):
                                o_both(tok)
                                return anchor(list(hold[0]) + list(hold[1]))
                            units.append((o_ab, L_A))
                            units.append((o_fin, L_C))
                        else:
                            def o_all(tok, o_both=o_both, o_fin=o_fin):
                                o_both(tok)
                                return o_fin(None)
                            units.append((o_all, 26))
            return units

        def stage_mm(vsrc, mdst, p0=0, p1=NPOS):
            mode = cfg.get('mm', 'full')
            for pos in range(p0, p1):
                if mode == 'full':
                    v = pltpu.bitcast(vsrc[pos], BF16)
                    u = pltpu.bitcast(u_ref[pos], BF16)
                    mdst[pos] = jax.lax.dot_general(v, u, (((1,), (1,)), ((), ())),
                                                    preferred_element_type=F32)
                else:
                    nsp = cfg.get('nsp', 4)
                    nw = C // nsp
                    for n in range(nsp):
                        if mode == 'n':
                            v = pltpu.bitcast(vsrc[pos + zsm[4 + n]], BF16)
                        else:
                            v = pltpu.bitcast(vsrc[pos], BF16)
                        u = pltpu.bitcast(u_ref[pos, pl.ds(n * nw // 2, nw // 2)], BF16)
                        mdst[pos, :, pl.ds(n * nw, nw)] = jax.lax.dot_general(
                            v, u, (((1,), (1,)), ((), ())), preferred_element_type=F32)

        def out_copy(s, g):
            img = _shr(s, 2) & 1
            chunk = s & 3
            return pltpu.make_async_copy(src.at[4 + img, pl.ds(chunk * RC, RC), g],
                                         ob_.at[img, pl.ds(chunk * RC, RC), :, pl.ds(g * LG, LG)],
                                         sems.at[32 + (s - 8) * NG + g])

        def x_copy(img, c, g, nrows, sem):
            return pltpu.make_async_copy(xb.at[img, pl.ds(c * nrows, nrows), :, pl.ds(g * LG, LG)],
                                         src.at[img, pl.ds(c * nrows, nrows), g], sems.at[sem])

        def w1_copy(k):
            return pltpu.make_async_copy(w1b.at[:, :, pl.ds(k * 32, 32)],
                                         wraw.at[0, :, :, pl.ds(k * 32, 32)], sems.at[16 + k])

        def w_block(conv, k):
            for kk in range(4):
                for cb in range(NG):
                    w_unit(conv, u_ref, pl.multiple_of(k * 32 + kk * 8, 8), cb)

        for c in range(NCH):
            for g in range(NG):
                x_copy(0, c, g, RC, c * NG + g).start()
        for k in range(8):
            w1_copy(k).start()
        cx1 = [x_copy(1, 0, g, H, 24 + g) for g in range(NG)]
        cwe = pltpu.make_async_copy(wemb_hbm, wembs, sems.at[28])
        cw2 = pltpu.make_async_copy(w2b, wraw.at[1], sems.at[29])
        for cp in cx1:
            cp.start()
        cwe.start()
        cw2.start()
        cxr = []
        if cfg.get('resx'):
            xres[0, H] = jnp.zeros((NG, TW, LG), U32)
            for img in range(2):
                for g in range(NG):
                    cxr.append(pltpu.make_async_copy(xb.at[img, :, :, pl.ds(g * LG, LG)],
                                                     xres.at[img, pl.ds(0, H), g], sems.at[64 + img * NG + g]))
            for cp in cxr:
                cp.start()

        shb[...] = jnp.zeros(shb.shape, F32)
        zsm[0] = NPOS
        zvr[...] = jnp.zeros((8, LG), U32)
        zsm[1] = H
        zsm[2] = NSL * NP
        for n in range(4):
            zsm[4 + n] = 0
        v0[NPOS] = jnp.zeros((MC // 2, C), U32)
        v1[NPOS] = jnp.zeros((MC // 2, C), U32)
        src[0, H] = jnp.zeros((NG, TW, LG), U32)
        gbt[0, 0] = g1_ref[...].astype(F32).reshape(1, C)
        gbt[0, 1] = be1_ref[...].astype(F32).reshape(1, C)
        gbt[1, 0] = g2_ref[...].astype(F32).reshape(1, C)
        gbt[1, 1] = be2_ref[...].astype(F32).reshape(1, C)
        zero = jnp.zeros((1, C), F32)
        embtab[0] = zero
        embtab[1] = zero

        def mz_body(pos, carry):
            m1[pos] = jnp.zeros((MC, C), F32)
            return carry
        jax.lax.fori_loop(0, NPOS, mz_body, 0)

        def xs_body(c, carry):
            for g in range(NG):
                x_copy(0, c, g, RC, c * NG + g).wait()
            x_stats(0, c * RC, RC, c)
            return carry
        jax.lax.fori_loop(0, NCH, xs_body, 0)
        gn_params(0)
        run_chains([in_chain(0, v0, None)], paced=False)

        def wt_body(k, carry):
            w1_copy(k).wait()
            w_block(0, k)
            return carry
        jax.lax.fori_loop(0, 8, wt_body, 0)

        def step(s, par):
            cur, nxt = par, 1 - par
            if cfg.get('gp') == 'pre':
                gn_params(jnp.minimum(_shr(s + 1, 2), 3))
            chs = []
            if not cfg.get('noout'):
                chs.append(out_chain(s - 1, mbuf[nxt]))
            if not cfg.get('noin'):
                chs.append(in_chain(jnp.minimum(s + 1, 15), vbuf[nxt], 'top' if par == 1 else 'bot'))
            run_chains(chs)
            stage_mm(vbuf[cur], mbuf[cur])
            if not cfg.get('gp'):
                gn_params(jnp.minimum(_shr(s + 2, 2), 3))

        def body(s, carry):
            @pl.when(s == 2)
            def _():
                for cp in cx1:
                    cp.wait()

                def xs1(c, cc):
                    x_stats(1, c * RC, RC, c)
                    return cc
                jax.lax.fori_loop(0, NCH, xs1, 0)
                cwe.wait()
                emb_stage()

            @pl.when(s == 8)
            def _():
                cw2.wait()
                for cp in cxr:
                    cp.wait()

                def wt2(k, cc):
                    w_block(1, k)
                    return cc
                jax.lax.fori_loop(0, 8, wt2, 0)

            if cfg.get('gp') == 'when':
                @pl.when(((s & 3) == 3) & (s < 15))
                def _():
                    gn_params(jnp.minimum(_shr(s + 1, 2), 3))

            jax.lax.cond((s & 1) == 0, lambda: step(s, 0), lambda: step(s, 1))

            if not cfg.get('nodma'):
                @pl.when(s >= 9)
                def _():
                    for g in range(NG):
                        out_copy(s - 1, g).start()
            return carry
        ns = cfg.get('ns', 16)
        jax.lax.fori_loop(0, ns, body, 0)
        if ns < 16:
            if ns <= 2:
                for cp in cx1:
                    cp.wait()
                cwe.wait()
            if ns <= 8:
                cw2.wait()
                for cp in cxr:
                    cp.wait()
            for s in range(8, ns - 1):
                for g in range(NG):
                    if not cfg.get('nodma'):
                        out_copy(s, g).wait()
            return

        last = out_chain(15, m1)
        nper = len(last) // NG
        for g in range(NG):
            run_chains([last[g * nper:(g + 1) * nper]], paced=False)
            out_copy(15, g).start()
        for s in range(8, 16):
            for g in range(NG):
                out_copy(s, g).wait()

    return kernel


_KERNEL = make_kernel({'gp': 'when', 'T': 13200})


@jax.jit
def pallas_standalone__adm_resblock__diffusion_kernel(x, t_emb, g1, be1, w1, w_emb, g2, be2, w2):
    xh = jnp.transpose(x, (0, 2, 3, 1))
    w1t = jnp.transpose(w1, (2, 3, 0, 1))
    w2t = jnp.transpose(w2, (2, 3, 0, 1))
    vm = pl.BlockSpec(memory_space=pltpu.VMEM)
    hb = pl.BlockSpec(memory_space=pl.ANY)
    out = pl.pallas_call(
        _KERNEL,
        out_shape=jax.ShapeDtypeStruct((B, H, W, C), BF16),
        in_specs=[hb, vm, vm, vm, hb, hb, vm, vm, hb],
        out_specs=hb,
        scratch_shapes=[
            pltpu.VMEM((2, 3, 3, C // 2, C), U32),
            pltpu.VMEM((EMB, C), BF16),
            pltpu.VMEM((NPOS, C // 2, C), U32),
            pltpu.VMEM((6, H + 1, NG, TW, LG), U32),
            pltpu.VMEM((NPOS + 1, MC // 2, C), U32),
            pltpu.VMEM((NPOS + 1, MC // 2, C), U32),
            pltpu.VMEM((NPOS, MC, C), F32),
            pltpu.VMEM((NPOS, MC, C), F32),
            pltpu.VMEM((NSL * NP + 1, SHR, LG), F32),
            pltpu.VMEM((2, 4, 2, 8, LG), F32),
            pltpu.VMEM((5, NCH, 2, 8, C), F32),
            pltpu.VMEM((4, 1, C), F32),
            pltpu.VMEM((2, 2, 1, C), F32),
            pltpu.VMEM((4, 2, 8, C), F32),
            pltpu.VMEM((2, H + 1, NG, TW, LG), U32),
            pltpu.VMEM((8, LG), U32),
            pltpu.VMEM((4, 8, LG), F32),
            pltpu.SMEM((8,), jnp.int32),
            pltpu.SemaphoreType.DMA((72,)),
        ],
        compiler_params=pltpu.CompilerParams(vmem_limit_bytes=120 * 2 ** 20),
    )(xh, t_emb, g1, be1, w1t, w_emb, g2, be2, w2t)
    return jnp.transpose(out, (0, 3, 1, 2))
```

```python
import functools
import jax
import jax.numpy as jnp
from jax.experimental import pallas as pl
from jax.experimental.pallas import tpu as pltpu

B, C, H, W, EMB = 2, 512, 64, 64, 1152
NG, LG = 4, 128
TH = 4
NP = 6
NPOS = NP * NP
TW = W // 2
CT = 4
MC = CT * (W // TH)
RC = CT * TH
NCH = H // RC
NR = RC + 2
EPS = 1e-5
F32 = jnp.float32
BF16 = jnp.bfloat16
U32 = jnp.uint32

PA, PB = 2.0 / 3.0, 1.5


def _g_matrix():
    pts = [0.0, PA, -PA, PB, -PB]
    g = []
    for i, p in enumerate(pts):
        den = 1.0
        for j, q in enumerate(pts):
            if j != i:
                den *= (p - q)
        g.append([1.0 / den, p / den, p * p / den])
    g.append([0.0, 0.0, 1.0])
    return g


GH = _g_matrix()


def _bt(d):
    a2, b2 = PA * PA, PB * PB
    d0, d1, d2, d3, d4, d5 = d
    p2 = b2 * d2
    aa = d4 - p2
    ra = PA * (d3 - b2 * d1)
    ab = d4 - a2 * d2
    rb = PB * (d3 - a2 * d1)
    t0 = (d0 + ab) - p2
    t5 = (d1 + d5) - (a2 + b2) * d3
    return [t0, aa + ra, aa - ra, ab + rb, ab - rb, t5]


def _at(m):
    m0, m1, m2, m3, m4, m5 = m
    sa, da = m1 + m2, m1 - m2
    sb, db = m3 + m4, m3 - m4
    y0 = (m0 + sa) + sb
    y1 = PA * da + PB * db
    y2 = (PA * PA) * sa + (PB * PB) * sb
    y3 = ((PA ** 3) * da + (PB ** 3) * db) + m5
    return [y0, y1, y2, y3]


def _gt(g0, g1, g2):
    out = [None] * NP
    out[0] = GH[0][0] * g0
    for pp in (1, 3):
        ev = GH[pp][0] * g0 + GH[pp][2] * g2
        od = GH[pp][1] * g1
        out[pp] = ev + od
        out[pp + 1] = ev - od
    out[5] = g2
    return out


def _unpack(w, idx):
    return pltpu.unpack_elementwise(w, index=idx, packed_dtype=BF16, unpacked_dtype=F32)


def _pack(lo, hi):
    return pltpu.pack_elementwise([lo, hi], packed_dtype=BF16)


def _gs(g):
    return slice(g * LG, (g + 1) * LG)


def _static(s):
    return isinstance(s, int)


def make_kernel(cfg):
    T_IN = cfg.get('TI', cfg.get('T', 9500))
    T_OUT = cfg.get('TO', cfg.get('T', 9500))
    L_R, L_H = cfg.get('L_R', 40), cfg.get('L_H', 22)
    L_A, L_C = cfg.get('L_A', 20), cfg.get('L_C', 26)
    NRB = 2

    def kernel(x_hbm, t_ref, g1_ref, be1_ref, w1_hbm, wemb_hbm, g2_ref, be2_ref, w2_hbm,
               out_hbm,
               wraw, wembs, u_ref, src, v0, v1, m0, m1, rbuf, stats, embtab, gbt, gnp, zvr, zsm, sems):
        vbuf = (v0, v1)
        mbuf = (m0, m1)
        xb = x_hbm.bitcast(U32)
        ob_ = out_hbm.bitcast(U32)
        w1b = w1_hbm.bitcast(U32)
        w2b = w2_hbm.bitcast(U32)

        def delay(tok_u32, cyc):
            t = pltpu.bitcast(tok_u32, F32)
            n, rem = divmod(cyc, 116)
            for _ in range(n):
                t = jnp.broadcast_to(jnp.sum(t, axis=1, keepdims=True), (8, LG))
            for _ in range(rem // 8):
                t = jnp.tanh(t)
            return t

        def run_chains(chains, paced=True):
            items = []
            for ci, (tt, ch) in enumerate(chains):
                n = len(ch)
                nat = sum(c[1] for c in ch)
                extra = max(0.0, (tt - nat) / n)
                for k, (fn, lat) in enumerate(ch):
                    items.append(((k + 0.5) / n, ci, fn, int(extra)))
            items.sort(key=lambda it: (it[0], it[1]))
            toks = [None] * len(chains)
            for _, ci, fn, d in items:
                raw = fn(toks[ci])
                toks[ci] = delay(raw, d) if paced else None

        def anchor(vals):
            b = [pltpu.bitcast(v, U32) for v in vals]
            while len(b) > 1:
                b = [b[i] | b[i + 1] if i + 1 < len(b) else b[i] for i in range(0, len(b), 2)]
            return b[0] & zvr[...]

        def inj(x, tok):
            return x if tok is None else x + tok

        def x_stats(img, row0, nrows, slot):
            for g in range(NG):
                a1 = jnp.zeros((TW, LG), F32)
                a2 = jnp.zeros((TW, LG), F32)
                for j in range(nrows):
                    w = src[img, row0 + j, g]
                    e, o = _unpack(w, 0), _unpack(w, 1)
                    a1 = a1 + (e + o)
                    a2 = a2 + (e * e + o * o)
                stats[img, slot, 0, :, _gs(g)] = a1.reshape(4, 8, LG).sum(axis=0)
                stats[img, slot, 1, :, _gs(g)] = a2.reshape(4, 8, LG).sum(axis=0)

        def w_unit(conv, ob, cb):
            raw = [[[None] * 3 for _ in range(3)] for _ in range(2)]
            for i in range(3):
                for j in range(3):
                    w = wraw[conv, i, j, pl.ds(ob, 8), _gs(cb)]
                    raw[0][i][j], raw[1][i][j] = _unpack(w, 0), _unpack(w, 1)
            for qs in ((0,), (1, 2), (3, 4), (5,)):
                wq = [[[None] * 3 for _ in qs] for _ in range(2)]
                for par in range(2):
                    for i in range(3):
                        r0_, r1_, r2_ = raw[par][i]
                        if qs == (0,):
                            wq[par][0][i] = GH[0][0] * r0_
                        elif qs == (5,):
                            wq[par][0][i] = r2_
                        else:
                            pp = qs[0]
                            ev = GH[pp][0] * r0_ + GH[pp][2] * r2_
                            od = GH[pp][1] * r1_
                            wq[par][0][i] = ev + od
                            wq[par][1][i] = ev - od
                for qi, q in enumerate(qs):
                    o0 = _gt(*wq[0][qi])
                    o1 = _gt(*wq[1][qi])
                    for p in range(NP):
                        u_ref[p * NP + q, pl.ds(ob, 8), _gs(cb)] = _pack(o0[p], o1[p])

        def w_block(conv, k, nrb):
            for kk in range(nrb):
                for cb in range(NG):
                    w_unit(conv, pl.multiple_of((k * nrb + kk) * 8, 8), cb)

        def emb_stage():
            t = t_ref[...].astype(F32)
            st = (t * jax.nn.sigmoid(t)).astype(BF16)
            emb = jnp.dot(st, wembs[...], preferred_element_type=F32)
            embtab[2] = emb[0:1]
            embtab[3] = emb[1:2]

        def gn_params(sidx):
            conv = sidx >> 1
            s1 = stats[sidx, 0, 0] + stats[sidx, 1, 0] + stats[sidx, 2, 0] + stats[sidx, 3, 0]
            s2 = stats[sidx, 0, 1] + stats[sidx, 1, 1] + stats[sidx, 2, 1] + stats[sidx, 3, 1]
            s1 = jnp.sum(s1, axis=0, keepdims=True)
            s2 = jnp.sum(s2, axis=0, keepdims=True)
            e = embtab[sidx]
            n = float(H * W)
            t1 = s1 + n * e
            t2 = s2 + (2.0 * e) * s1 + (n * e) * e
            gam = gbt[conv, 0]
            bet = gbt[conv, 1]
            inv = 1.0 / (H * W * LG)
            for g in range(NG):
                mean = jnp.sum(t1[:, _gs(g)], axis=1, keepdims=True) * inv
                ex2 = jnp.sum(t2[:, _gs(g)], axis=1, keepdims=True) * inv
                var = jnp.maximum(ex2 - mean * mean, 0.0)
                rstd = jax.lax.rsqrt(var + EPS)
                sc = gam[:, _gs(g)] * rstd
                sh = bet[:, _gs(g)] + (e[:, _gs(g)] - mean) * sc
                gnp[sidx, 0, :, _gs(g)] = jnp.broadcast_to(0.5 * sc, (8, LG))
                gnp[sidx, 1, :, _gs(g)] = jnp.broadcast_to(0.5 * sh, (8, LG))

        def in_chain(s, vdst, edge):
            sidx = s >> 2
            chunk = s & 3
            r0 = chunk * RC - 1
            sub = jax.lax.broadcasted_iota(jnp.int32, (8, LG), 0)
            units = []
            for g in range(NG):
                base = (g % NRB) * NR * 12

                def row_link(tok, g=g, base=base, lr=0):
                    r = r0 + lr
                    valid = None
                    zero_row = False
                    if _static(r):
                        zero_row = r < 0 or r >= H
                    elif lr == 0 and edge in ('top', 'both'):
                        valid = r >= 0
                        r = jnp.maximum(r, 0)
                    elif lr == NR - 1 and edge in ('bot', 'both'):
                        valid = r < H
                        r = jnp.minimum(r, H - 1)
                    if zero_row:
                        z = jnp.zeros((8, LG), F32)
                        for q in range(12):
                            rbuf[base + lr * 12 + q] = z
                    else:
                        sc = inj(gnp[sidx, 0, :, _gs(g)], tok)
                        sh = gnp[sidx, 1, :, _gs(g)]
                        c = []
                        for j in range(4):
                            w = src[sidx, r, g, pl.ds(j, 8, stride=4), :]
                            for half in range(2):
                                hv = _unpack(w, half) * sc + sh
                                a = hv + hv * jnp.tanh(hv)
                                if valid is not None:
                                    a = jnp.where(valid, a, 0.0)
                                c.append(a)
                        left = jnp.where(sub == 0, 0.0, pltpu.roll(c[7], 1, 0))
                        right = jnp.where(sub == 7, 0.0, pltpu.roll(c[0], 7, 0))
                        ev = _bt([left, c[0], c[1], c[2], c[3], c[4]])
                        od = _bt([c[3], c[4], c[5], c[6], c[7], right])
                        for q in range(NP):
                            rbuf[base + lr * 12 + q] = ev[q]
                            rbuf[base + lr * 12 + 6 + q] = od[q]
                    return pltpu.bitcast(rbuf[zsm[2]], U32)

                def col_link(tok, g=g, base=base, ty=0, q=0):
                    t = []
                    for par in range(2):
                        d = [rbuf[base + (ty * TH + i) * 12 + 6 * par + q] for i in range(NP)]
                        if par == 0:
                            d[2] = inj(d[2], tok)
                        t.append(_bt(d))
                    for p in range(NP):
                        vdst[p * NP + q, pl.ds(ty * 8, 8), _gs(g)] = _pack(t[0][p], t[1][p])
                    return vdst[zsm[0], 0:8, 0:LG]

                for ty in range(CT):
                    for lr in range(0 if ty == 0 else ty * TH + 2, ty * TH + NP):
                        units.append((functools.partial(row_link, lr=lr), L_R))
                    for q in range(NP):
                        units.append((functools.partial(col_link, ty=ty, q=q), L_H))
            return units

        def out_chain(s, msrc):
            img = (s >> 2) & 1
            chunk = s & 3
            kind2 = s >= 8
            if _static(s):
                dslot = (4 if kind2 else 2) + img
                sslot = 4 if kind2 else 2 + img
                rslot = img if kind2 else 0
            else:
                dslot = jnp.where(kind2, 4, 2) + img
                sslot = jnp.where(kind2, 4, 2 + img)
                rslot = jnp.where(kind2, img, 0)
            need_stats = not (_static(s) and kind2)
            units = []
            for g in range(NG):
                acc = [jnp.zeros((8, LG), F32), jnp.zeros((8, LG), F32)]
                for b in range(2 * CT):
                    hold = {}

                    def w_link(tok, g=g, b=b, hold=hold, ps=()):
                        vals = []
                        for p in ps:
                            mm = [msrc[p * NP + q, pl.ds(8 * b, 8), _gs(g)] for q in range(NP)]
                            if p == ps[0]:
                                mm[1] = inj(mm[1], tok)
                            hold[p] = _at(mm)
                            vals += hold[p]
                        return anchor(vals)

                    def fin_link(tok, g=g, b=b, acc=acc, hold=hold, e=0):
                        ty, hh = b // 2, b % 2
                        xw = []
                        for k in range(TH):
                            r = chunk * RC + ty * TH + k
                            if _static(s):
                                rr = r if kind2 else H
                            else:
                                rr = jnp.where(kind2, r, H)
                            xw.append(src[rslot, rr, g, pl.ds(16 * hh + e, 8, stride=2), :])
                        y = []
                        for l in (2 * e, 2 * e + 1):
                            col = [hold[p][l] for p in range(NP)]
                            col[1] = inj(col[1], tok)
                            y.append(_at(col))
                        for k in range(TH):
                            r = chunk * RC + ty * TH + k
                            ye, yo = y[0][k], y[1][k]
                            if need_stats:
                                acc[0] = acc[0] + (ye + yo)
                                acc[1] = acc[1] + (ye * ye + yo * yo)
                            src[dslot, r, g, pl.ds(16 * hh + e, 8, stride=2), :] = _pack(
                                ye + _unpack(xw[k], 0), yo + _unpack(xw[k], 1))
                        if need_stats and b == 2 * CT - 1 and e == 1:
                            stats[sslot, chunk, 0, :, _gs(g)] = acc[0]
                            stats[sslot, chunk, 1, :, _gs(g)] = acc[1]
                        tk = src[0, zsm[1], 0, 0:8, :]
                        if need_stats:
                            tk = tk | anchor(acc)
                        return tk

                    units.append((functools.partial(w_link, ps=(0, 1, 2)), L_A))
                    units.append((functools.partial(w_link, ps=(3, 4, 5)), L_A))
                    units.append((functools.partial(fin_link, e=0), L_C))
                    units.append((functools.partial(fin_link, e=1), L_C))
            return units

        def stage_mm(vsrc, mdst):
            for pos in range(NPOS):
                v = pltpu.bitcast(vsrc[pos], BF16)
                u = pltpu.bitcast(u_ref[pos], BF16)
                mdst[pos] = jax.lax.dot_general(v, u, (((1,), (1,)), ((), ())),
                                                preferred_element_type=F32)

        def out_copy(s, g):
            img = (s >> 2) & 1
            chunk = s & 3
            return pltpu.make_async_copy(src.at[4 + img, pl.ds(chunk * RC, RC), g],
                                         ob_.at[img, pl.ds(chunk * RC, RC), :, pl.ds(g * LG, LG)],
                                         sems.at[48 + (s - 8) * NG + g])

        def x_copy(img, c, g, nrows, sem):
            return pltpu.make_async_copy(xb.at[img, pl.ds(c * nrows, nrows), :, pl.ds(g * LG, LG)],
                                         src.at[img, pl.ds(c * nrows, nrows), g], sems.at[sem])

        NW1 = cfg.get('NW1', 16)
        WR = (C // 2) // NW1

        def w1_copy(k):
            return pltpu.make_async_copy(w1b.at[:, :, pl.ds(k * WR, WR)],
                                         wraw.at[0, :, :, pl.ds(k * WR, WR)], sems.at[16 + k])

        for c in range(NCH):
            for g in range(NG):
                x_copy(0, c, g, RC, c * NG + g).start()
        for k in range(NW1):
            w1_copy(k).start()
        cx1 = [x_copy(1, 0, g, H, 32 + g) for g in range(NG)]
        cwe = pltpu.make_async_copy(wemb_hbm, wembs, sems.at[36])
        cw2 = pltpu.make_async_copy(w2b, wraw.at[1], sems.at[37])
        for cp in cx1:
            cp.start()
        cwe.start()
        cw2.start()

        zsm[0] = NPOS
        zsm[1] = H
        zsm[2] = NRB * NR * 12
        zvr[...] = jnp.zeros((8, LG), U32)
        rbuf[NRB * NR * 12] = jnp.zeros((8, LG), F32)
        v0[NPOS] = jnp.zeros((MC // 2, C), U32)
        v1[NPOS] = jnp.zeros((MC // 2, C), U32)
        src[0, H] = jnp.zeros((NG, TW, LG), U32)
        gbt[0, 0] = g1_ref[...].astype(F32).reshape(1, C)
        gbt[0, 1] = be1_ref[...].astype(F32).reshape(1, C)
        gbt[1, 0] = g2_ref[...].astype(F32).reshape(1, C)
        gbt[1, 1] = be2_ref[...].astype(F32).reshape(1, C)
        zero = jnp.zeros((1, C), F32)
        embtab[0] = zero
        embtab[1] = zero

        def mz_body(pos, carry):
            m1[pos] = jnp.zeros((MC, C), F32)
            return carry
        jax.lax.fori_loop(0, NPOS, mz_body, 0)

        def xs_body(c, carry):
            for g in range(NG):
                x_copy(0, c, g, RC, c * NG + g).wait()
            x_stats(0, c * RC, RC, c)
            return carry
        jax.lax.fori_loop(0, NCH, xs_body, 0)
        gn_params(0)
        run_chains([(0, in_chain(0, v0, None))], paced=False)

        def wt_body(k, carry):
            w1_copy(k).wait()
            w_block(0, k, WR // 8)
            return carry
        jax.lax.fori_loop(0, NW1, wt_body, 0)

        def step(s, par):
            cur, nxt = par, 1 - par
            chs = []
            if not cfg.get('noout'):
                chs.append((T_OUT, out_chain(s - 1, mbuf[nxt])))
            if not cfg.get('noin'):
                chs.append((T_IN, in_chain(jnp.minimum(s + 1, 15), vbuf[nxt], 'top' if par == 1 else 'bot')))
            run_chains(chs)
            stage_mm(vbuf[cur], mbuf[cur])

        def body(s, carry):
            @pl.when(s == 2)
            def _():
                for cp in cx1:
                    cp.wait()

                def xs1(c, cc):
                    x_stats(1, c * RC, RC, c)
                    return cc
                jax.lax.fori_loop(0, NCH, xs1, 0)

            @pl.when(s == 3)
            def _():
                cwe.wait()
                emb_stage()
                gn_params(1)

            @pl.when((s == 7) | (s == 11))
            def _():
                gn_params((s + 1) >> 2)

            @pl.when(s == 8)
            def _():
                cw2.wait()

                def wt2(k, cc):
                    w_block(1, k, 2)
                    return cc
                jax.lax.fori_loop(0, C // 32, wt2, 0)

            jax.lax.cond((s & 1) == 0, lambda: step(s, 0), lambda: step(s, 1))

            @pl.when(s >= 9)
            def _():
                for g in range(NG):
                    out_copy(s - 1, g).start()
            return carry

        ns = cfg.get('ns', 16)
        jax.lax.fori_loop(0, ns, body, 0)
        if ns < 16:
            if ns <= 2:
                for cp in cx1:
                    cp.wait()
            if ns <= 3:
                cwe.wait()
            if ns <= 8:
                cw2.wait()
            for s in range(8, ns - 1):
                for g in range(NG):
                    out_copy(s, g).wait()
            return

        last = out_chain(15, m1)
        nper = len(last) // NG
        for g in range(NG):
            run_chains([(0, last[g * nper:(g + 1) * nper])], paced=False)
            out_copy(15, g).start()
        for s in range(8, 16):
            for g in range(NG):
                out_copy(s, g).wait()

    return kernel


_KERNEL = make_kernel({'T': 9500})


@jax.jit
def pallas_standalone__adm_resblock__diffusion_kernel(x, t_emb, g1, be1, w1, w_emb, g2, be2, w2):
    xh = jnp.transpose(x, (0, 2, 3, 1))
    w1t = jnp.transpose(w1, (2, 3, 0, 1))
    w2t = jnp.transpose(w2, (2, 3, 0, 1))
    vm = pl.BlockSpec(memory_space=pltpu.VMEM)
    hb = pl.BlockSpec(memory_space=pl.ANY)
    out = pl.pallas_call(
        _KERNEL,
        out_shape=jax.ShapeDtypeStruct((B, H, W, C), BF16),
        in_specs=[hb, vm, vm, vm, hb, hb, vm, vm, hb],
        out_specs=hb,
        scratch_shapes=[
            pltpu.VMEM((2, 3, 3, C // 2, C), U32),
            pltpu.VMEM((EMB, C), BF16),
            pltpu.VMEM((NPOS, C // 2, C), U32),
            pltpu.VMEM((6, H + 1, NG, TW, LG), U32),
            pltpu.VMEM((NPOS + 1, MC // 2, C), U32),
            pltpu.VMEM((NPOS + 1, MC // 2, C), U32),
            pltpu.VMEM((NPOS, MC, C), F32),
            pltpu.VMEM((NPOS, MC, C), F32),
            pltpu.VMEM((2 * NR * 12 + 1, 8, LG), F32),
            pltpu.VMEM((5, NCH, 2, 8, C), F32),
            pltpu.VMEM((4, 1, C), F32),
            pltpu.VMEM((2, 2, 1, C), F32),
            pltpu.VMEM((4, 2, 8, C), F32),
            pltpu.VMEM((8, LG), U32),
            pltpu.SMEM((8,), jnp.int32),
            pltpu.SemaphoreType.DMA((80,)),
        ],
        compiler_params=pltpu.CompilerParams(vmem_limit_bytes=120 * 2 ** 20),
    )(xh, t_emb, g1, be1, w1t, w_emb, g2, be2, w2t)
    return jnp.transpose(out, (0, 3, 1, 2))
```

```python
import functools
import jax
import jax.numpy as jnp
from jax.experimental import pallas as pl
from jax.experimental.pallas import tpu as pltpu

B, C, H, W, EMB = 2, 512, 64, 64, 1152
NG, LG = 4, 128
TH = 4
NP = 6
NPOS = NP * NP
TW = W // 2
CT = 4
MC = CT * (W // TH)
RC = CT * TH
NCH = H // RC
NR = RC + 2
EPS = 1e-5
F32 = jnp.float32
BF16 = jnp.bfloat16
U32 = jnp.uint32

PA, PB = 2.0 / 3.0, 1.5


CA = 1.0 / (2.0 * PA * PA * (PA * PA - PB * PB))
CB = 1.0 / (PA * PA * 2.0 * PB * PB * (PB * PB - PA * PA))


def _bt(d):
    a2, b2 = PA * PA, PB * PB
    d0, d1, d2, d3, d4, d5 = d
    p2 = b2 * d2
    aa = d4 - p2
    ra = PA * (d3 - b2 * d1)
    ab = d4 - a2 * d2
    rb = PB * (d3 - a2 * d1)
    t0 = (d0 + ab) - p2
    t5 = (d1 + d5) - (a2 + b2) * d3
    return [t0, aa + ra, aa - ra, ab + rb, ab - rb, t5]


def _at(m):
    m0, m1, m2, m3, m4, m5 = m
    sa, da = m1 + m2, m1 - m2
    sb, db = m3 + m4, m3 - m4
    y0 = (m0 + CA * sa) + CB * sb
    y1 = (CA * PA) * da + (CB * PB) * db
    y2 = (CA * PA * PA) * sa + (CB * PB * PB) * sb
    y3 = ((CA * PA ** 3) * da + (CB * PB ** 3) * db) + m5
    return [y0, y1, y2, y3]


def _gt(g0, g1, g2):
    a2 = PA * PA
    od = PA * g1
    ea = g0 + a2 * g2
    eb = a2 * g0 + g2
    return [g0, ea + od, ea - od, eb + od, eb - od, g2]


def _unpack(w, idx):
    return pltpu.unpack_elementwise(w, index=idx, packed_dtype=BF16, unpacked_dtype=F32)


def _pack(lo, hi):
    return pltpu.pack_elementwise([lo, hi], packed_dtype=BF16)


def _gs(g):
    return slice(g * LG, (g + 1) * LG)


def _static(s):
    return isinstance(s, int)


def make_kernel(cfg):
    T_IN = cfg.get('TI', cfg.get('T', 9500))
    T_OUT = cfg.get('TO', cfg.get('T', 9500))
    L_R, L_H = cfg.get('L_R', 40), cfg.get('L_H', 22)
    L_A, L_C = cfg.get('L_A', 20), cfg.get('L_C', 26)
    L_U, T_U, URB = cfg.get('L_U', 30), cfg.get('TU', cfg.get('T', 9500)), cfg.get('URB', 5)
    NRB = 2

    def kernel(x_hbm, t_hbm, g1_hbm, be1_hbm, w1_hbm, wemb_hbm, g2_hbm, be2_hbm, w2_hbm,
               out_hbm,
               t_ref, g1_ref, be1_ref, g2_ref, be2_ref,
               wraw, wembs, u_ref, u2_ref, src, v0, v1, m0, m1, rbuf, stats, embtab, gbt, gnp, zvr, zsm, sems):
        vbuf = (v0, v1)
        mbuf = (m0, m1)
        xb = x_hbm.bitcast(U32)
        ob_ = out_hbm.bitcast(U32)
        w1b = w1_hbm.bitcast(U32)
        w2b = w2_hbm.bitcast(U32)

        def delay(tok_u32, cyc):
            t = pltpu.bitcast(tok_u32, F32)
            n, rem = divmod(cyc, 116)
            for _ in range(n):
                t = jnp.broadcast_to(jnp.sum(t, axis=1, keepdims=True), (8, LG))
            for _ in range(rem // 8):
                t = jnp.tanh(t)
            return t

        def run_chains(chains, paced=True):
            items = []
            for ci, (tt, ch) in enumerate(chains):
                n = len(ch)
                nat = sum(c[1] for c in ch)
                extra = max(0.0, (tt - nat) / n)
                for k, (fn, lat) in enumerate(ch):
                    items.append(((k + 0.5) / n, ci, fn, int(extra)))
            items.sort(key=lambda it: (it[0], it[1]))
            toks = [None] * len(chains)
            for _, ci, fn, d in items:
                raw = fn(toks[ci])
                toks[ci] = delay(raw, d) if paced else None

        def anchor(vals):
            b = [pltpu.bitcast(v, U32) for v in vals]
            while len(b) > 1:
                b = [b[i] | b[i + 1] if i + 1 < len(b) else b[i] for i in range(0, len(b), 2)]
            return b[0] & zvr[...]

        def inj(x, tok):
            return x if tok is None else x + tok

        def x_stats(img, row0, nrows, slot):
            for g in range(NG):
                a1 = [jnp.zeros((8, LG), F32)] * 2
                a2 = [jnp.zeros((8, LG), F32)] * 2
                for j in range(nrows):
                    for t in range(TW // 8):
                        w = src[img, row0 + j, g, pl.ds(8 * t, 8), :]
                        e, o = _unpack(w, 0), _unpack(w, 1)
                        a1[t % 2] = a1[t % 2] + (e + o)
                        a2[t % 2] = a2[t % 2] + (e * e + o * o)
                stats[img, slot, 0, :, _gs(g)] = a1[0] + a1[1]
                stats[img, slot, 1, :, _gs(g)] = a2[0] + a2[1]

        def w_unit(conv, ob, cb):
            raw = [[[None] * 3 for _ in range(3)] for _ in range(2)]
            for i in range(3):
                for j in range(3):
                    w = wraw[conv, i, j, pl.ds(ob, 8), _gs(cb)]
                    raw[0][i][j], raw[1][i][j] = _unpack(w, 0), _unpack(w, 1)
            wq = [[_gt(*raw[par][i]) for i in range(3)] for par in range(2)]
            for q in range(NP):
                o0 = _gt(*[wq[0][i][q] for i in range(3)])
                o1 = _gt(*[wq[1][i][q] for i in range(3)])
                for p in range(NP):
                    u_ref[p * NP + q, pl.ds(ob, 8), _gs(cb)] = _pack(o0[p], o1[p])

        def w_block(conv, k, nrb):
            for kk in range(nrb):
                for cb in range(NG):
                    w_unit(conv, pl.multiple_of((k * nrb + kk) * 8, 8), cb)

        def u_chain(s):
            cv = jnp.where(s < 1, 0, 1)
            a2 = PA * PA
            units = []
            for kk in range(URB):
                rb = jnp.minimum(jnp.maximum(s - 1, 0) * URB + kk, C // 16 - 1)
                ob = pl.multiple_of(rb * 8, 8)
                for cb in range(NG):
                    def u_link(tok, ob=ob, cb=cb, qs=()):
                        js = (0,) if qs == (0,) else (2,) if qs == (5,) else (0, 1, 2)
                        wq = [[], []]
                        for i in range(3):
                            w = [wraw[cv, i, j, pl.ds(ob, 8), _gs(cb)] for j in js]
                            for par in range(2):
                                r = [_unpack(x, par) for x in w]
                                if par == 0:
                                    r[0] = inj(r[0], tok)
                                if len(js) == 1:
                                    wq[par].append(r)
                                else:
                                    od = PA * r[1]
                                    ev = r[0] + a2 * r[2] if qs == (1, 2) else a2 * r[0] + r[2]
                                    wq[par].append([ev + od, ev - od])
                        for qi, q in enumerate(qs):
                            o0 = _gt(*[wq[0][i][qi] for i in range(3)])
                            o1 = _gt(*[wq[1][i][qi] for i in range(3)])
                            for p in range(NP):
                                u2_ref[p * NP + q, pl.ds(ob, 8), _gs(cb)] = _pack(o0[p], o1[p])
                        return u2_ref[zsm[0], 0:8, 0:LG]

                    units.append((functools.partial(u_link, qs=(0,)), L_U // 2))
                    units.append((functools.partial(u_link, qs=(1, 2)), L_U))
                    units.append((functools.partial(u_link, qs=(3, 4)), L_U))
                    units.append((functools.partial(u_link, qs=(5,)), L_U // 2))
            return units

        def emb_stage():
            t = t_ref[...].astype(F32)
            st = (t * jax.nn.sigmoid(t)).astype(BF16)
            emb = jnp.dot(st, wembs[...], preferred_element_type=F32)
            embtab[2] = emb[0:1]
            embtab[3] = emb[1:2]

        def gn_params(sidx):
            conv = sidx >> 1
            s1 = stats[sidx, 0, 0] + stats[sidx, 1, 0] + stats[sidx, 2, 0] + stats[sidx, 3, 0]
            s2 = stats[sidx, 0, 1] + stats[sidx, 1, 1] + stats[sidx, 2, 1] + stats[sidx, 3, 1]
            s1 = jnp.sum(s1, axis=0, keepdims=True)
            s2 = jnp.sum(s2, axis=0, keepdims=True)
            e = embtab[sidx]
            n = float(H * W)
            t1 = s1 + n * e
            t2 = s2 + (2.0 * e) * s1 + (n * e) * e
            gam = gbt[conv, 0]
            bet = gbt[conv, 1]
            inv = 1.0 / (H * W * LG)
            for g in range(NG):
                mean = jnp.sum(t1[:, _gs(g)], axis=1, keepdims=True) * inv
                ex2 = jnp.sum(t2[:, _gs(g)], axis=1, keepdims=True) * inv
                var = jnp.maximum(ex2 - mean * mean, 0.0)
                rstd = jax.lax.rsqrt(var + EPS)
                sc = gam[:, _gs(g)] * rstd
                sh = bet[:, _gs(g)] + (e[:, _gs(g)] - mean) * sc
                gnp[sidx, 0, :, _gs(g)] = jnp.broadcast_to(0.5 * sc, (8, LG))
                gnp[sidx, 1, :, _gs(g)] = jnp.broadcast_to(0.5 * sh, (8, LG))

        def in_chain(s, vdst, edge):
            sidx = s >> 2
            chunk = s & 3
            r0 = chunk * RC - 1
            sub = jax.lax.broadcasted_iota(jnp.int32, (8, LG), 0)
            units = []
            for g in range(NG):
                base = (g % NRB) * NR * 12

                def row_link(tok, g=g, base=base, lr=0):
                    r = r0 + lr
                    valid = None
                    zero_row = False
                    if _static(r):
                        zero_row = r < 0 or r >= H
                    elif lr == 0 and edge in ('top', 'both'):
                        valid = r >= 0
                        r = jnp.maximum(r, 0)
                    elif lr == NR - 1 and edge in ('bot', 'both'):
                        valid = r < H
                        r = jnp.minimum(r, H - 1)
                    if zero_row:
                        z = jnp.zeros((8, LG), F32)
                        for q in range(12):
                            rbuf[base + lr * 12 + q] = z
                    else:
                        sc = inj(gnp[sidx, 0, :, _gs(g)], tok)
                        sh = gnp[sidx, 1, :, _gs(g)]
                        c = []
                        for j in range(4):
                            w = src[sidx, r, g, pl.ds(j, 8, stride=4), :]
                            for half in range(2):
                                hv = _unpack(w, half) * sc + sh
                                a = hv + hv * jnp.tanh(hv)
                                if valid is not None:
                                    a = jnp.where(valid, a, 0.0)
                                c.append(a)
                        left = jnp.where(sub == 0, 0.0, pltpu.roll(c[7], 1, 0))
                        right = jnp.where(sub == 7, 0.0, pltpu.roll(c[0], 7, 0))
                        ev = _bt([left, c[0], c[1], c[2], c[3], c[4]])
                        od = _bt([c[3], c[4], c[5], c[6], c[7], right])
                        for q in range(NP):
                            rbuf[base + lr * 12 + q] = ev[q]
                            rbuf[base + lr * 12 + 6 + q] = od[q]
                    return pltpu.bitcast(rbuf[zsm[2]], U32)

                def col_link(tok, g=g, base=base, ty=0, q=0):
                    t = []
                    for par in range(2):
                        d = [rbuf[base + (ty * TH + i) * 12 + 6 * par + q] for i in range(NP)]
                        if par == 0:
                            d[2] = inj(d[2], tok)
                        t.append(_bt(d))
                    for p in range(NP):
                        vdst[p * NP + q, pl.ds(ty * 8, 8), _gs(g)] = _pack(t[0][p], t[1][p])
                    return vdst[zsm[0], 0:8, 0:LG]

                for ty in range(CT):
                    for lr in range(0 if ty == 0 else ty * TH + 2, ty * TH + NP):
                        units.append((functools.partial(row_link, lr=lr), L_R))
                    for q in range(NP):
                        units.append((functools.partial(col_link, ty=ty, q=q), L_H))
            return units

        def out_chain(s, msrc, conv1=False):
            img = (s >> 2) & 1
            chunk = s & 3
            kind2 = False if conv1 else s >= 8
            if conv1:
                dslot, sslot, rslot = 2 + img, 2 + img, 0
            elif _static(s):
                dslot = (4 if kind2 else 2) + img
                sslot = 4 if kind2 else 2 + img
                rslot = img if kind2 else 0
            else:
                dslot = jnp.where(kind2, 4, 2) + img
                sslot = jnp.where(kind2, 4, 2 + img)
                rslot = jnp.where(kind2, img, 0)
            need_stats = not (_static(s) and kind2)
            units = []
            for g in range(NG):
                acc = [jnp.zeros((8, LG), F32), jnp.zeros((8, LG), F32)]
                for b in range(2 * CT):
                    hold = {}

                    def w_link(tok, g=g, b=b, hold=hold, ps=()):
                        vals = []
                        for p in ps:
                            mm = [msrc[p * NP + q, pl.ds(8 * b, 8), _gs(g)] for q in range(NP)]
                            if p == ps[0]:
                                mm[1] = inj(mm[1], tok)
                            hold[p] = _at(mm)
                            vals += hold[p]
                        return anchor(vals)

                    def fin_link(tok, g=g, b=b, acc=acc, hold=hold, e=0):
                        ty, hh = b // 2, b % 2
                        xw = []
                        for k in range(0 if conv1 else TH):
                            r = chunk * RC + ty * TH + k
                            if _static(s):
                                rr = r if kind2 else H
                            else:
                                rr = jnp.where(kind2, r, H)
                            xw.append(src[rslot, rr, g, pl.ds(16 * hh + e, 8, stride=2), :])
                        y = []
                        for l in (2 * e, 2 * e + 1):
                            col = [hold[p][l] for p in range(NP)]
                            col[1] = inj(col[1], tok)
                            y.append(_at(col))
                        for k in range(TH):
                            r = chunk * RC + ty * TH + k
                            ye, yo = y[0][k], y[1][k]
                            if need_stats:
                                acc[0] = acc[0] + (ye + yo)
                                acc[1] = acc[1] + (ye * ye + yo * yo)
                            if not conv1:
                                ye, yo = ye + _unpack(xw[k], 0), yo + _unpack(xw[k], 1)
                            src[dslot, r, g, pl.ds(16 * hh + e, 8, stride=2), :] = _pack(ye, yo)
                        if need_stats and b == 2 * CT - 1 and e == 1:
                            stats[sslot, chunk, 0, :, _gs(g)] = acc[0]
                            stats[sslot, chunk, 1, :, _gs(g)] = acc[1]
                        tk = src[0, zsm[1], 0, 0:8, :]
                        if need_stats:
                            tk = tk | anchor(acc)
                        return tk

                    units.append((functools.partial(w_link, ps=(0, 1, 2)), L_A))
                    units.append((functools.partial(w_link, ps=(3, 4, 5)), L_A))
                    units.append((functools.partial(fin_link, e=0), L_C))
                    units.append((functools.partial(fin_link, e=1), L_C))
            return units

        def stage_mm(vsrc, mdst, usrc):
            for pos in range(NPOS):
                v = pltpu.bitcast(vsrc[pos], BF16)
                u = pltpu.bitcast(usrc[pos], BF16)
                mdst[pos] = jax.lax.dot_general(v, u, (((1,), (1,)), ((), ())),
                                                preferred_element_type=F32)

        def out_copy(s, g):
            img = (s >> 2) & 1
            chunk = s & 3
            return pltpu.make_async_copy(src.at[4 + img, pl.ds(chunk * RC, RC), g],
                                         ob_.at[img, pl.ds(chunk * RC, RC), :, pl.ds(g * LG, LG)],
                                         sems.at[48 + (s - 8) * NG + g])

        def x_copy(img, c, g, nrows, sem):
            return pltpu.make_async_copy(xb.at[img, pl.ds(c * nrows, nrows), :, pl.ds(g * LG, LG)],
                                         src.at[img, pl.ds(c * nrows, nrows), g], sems.at[sem])

        NW1 = cfg.get('NW1', 16)
        WR = (C // 2) // NW1

        def w1_copy(k):
            return pltpu.make_async_copy(w1b.at[:, :, pl.ds(k * WR, WR)],
                                         wraw.at[0, :, :, pl.ds(k * WR, WR)], sems.at[16 + k])

        for c in range(NCH):
            for g in range(NG):
                x_copy(0, c, g, RC, c * NG + g).start()
        small = [pltpu.make_async_copy(a, b, sems.at[40 + i]) for i, (a, b) in enumerate(
            ((g1_hbm, g1_ref), (be1_hbm, be1_ref), (g2_hbm, g2_ref), (be2_hbm, be2_ref), (t_hbm, t_ref)))]
        for cp in small:
            cp.start()
        for k in range(NW1 if cfg.get('dmaonly') != 1 else 0):
            w1_copy(k).start()
        cx1 = [x_copy(1, 0, g, H, 32 + g) for g in range(NG)]
        cwe = pltpu.make_async_copy(wemb_hbm, wembs, sems.at[36])
        cw2 = pltpu.make_async_copy(w2b, wraw.at[1], sems.at[37])
        nod2 = cfg.get('nod2')
        if not nod2:
            cw2.start()
            for cp in cx1:
                cp.start()
            cwe.start()

        zsm[0] = NPOS
        zsm[1] = H
        zsm[2] = NRB * NR * 12
        zsm[3] = 0
        zvr[...] = jnp.zeros((8, LG), U32)
        rbuf[NRB * NR * 12] = jnp.zeros((8, LG), F32)
        v0[NPOS] = jnp.zeros((MC // 2, C), U32)
        v1[NPOS] = jnp.zeros((MC // 2, C), U32)
        u2_ref[NPOS, 0:8, 0:LG] = jnp.zeros((8, LG), U32)
        src[0, H] = jnp.zeros((NG, TW, LG), U32)
        zero = jnp.zeros((1, C), F32)
        embtab[0] = zero
        embtab[1] = zero

        def mz_body(pos, carry):
            m1[pos] = jnp.zeros((MC, C), F32)
            return carry
        jax.lax.fori_loop(0, NPOS, mz_body, 0)

        if cfg.get('dum'):
            @pl.when(zsm[3] == 1)
            def _():
                for pos in range(cfg['dum']):
                    u_ref[pos] = jnp.full((C // 2, C), pos + 1, U32)

        def xs_body(c, carry):
            for g in range(NG):
                x_copy(0, c, g, RC, c * NG + g).wait()
            x_stats(0, c * RC, RC, c)
            return carry

        def wt_body(k, carry):
            w1_copy(k).wait()
            w_block(0, k, WR // 8)
            return carry

        def prologue():
            if cfg.get('dmaonly'):
                for c in range(NCH):
                    for g in range(NG):
                        x_copy(0, c, g, RC, c * NG + g).wait()
                for cp in small:
                    cp.wait()
                if cfg['dmaonly'] == 2:
                    for k in range(NW1):
                        w1_copy(k).wait()
                return
            jax.lax.fori_loop(0, NCH, xs_body, 0)
            for cp in small:
                cp.wait()
            gbt[0, 0] = g1_ref[...].astype(F32).reshape(1, C)
            gbt[0, 1] = be1_ref[...].astype(F32).reshape(1, C)
            gbt[1, 0] = g2_ref[...].astype(F32).reshape(1, C)
            gbt[1, 1] = be2_ref[...].astype(F32).reshape(1, C)
            gn_params(0)
            run_chains([(0, in_chain(0, v0, None))], paced=False)
            jax.lax.fori_loop(0, NW1, wt_body, 0)

        if not cfg.get('pin'):
            prologue()

        def step(s, par, conv1):
            cur, nxt = par, 1 - par
            t_out, t_in = (cfg.get('TO1', T_OUT), cfg.get('TI1', T_IN)) if conv1 else (T_OUT, T_IN)
            chs = [(t_out, out_chain(s - 1, mbuf[nxt], conv1)),
                   (t_in, in_chain(jnp.minimum(s + 1, 15), vbuf[nxt], 'top' if par == 1 else 'bot'))]
            if conv1:
                chs.append((T_U, u_chain(s)))
            run_chains(chs)
            stage_mm(vbuf[cur], mbuf[cur], u_ref if conv1 else u2_ref)

        def body1(s, carry):
            @pl.when(s == 1)
            def _():
                cw2.wait()

            @pl.when(s == 2)
            def _():
                for cp in cx1:
                    cp.wait()

                def xs1(c, cc):
                    x_stats(1, c * RC, RC, c)
                    return cc
                jax.lax.fori_loop(0, NCH, xs1, 0)

            @pl.when(s == 3)
            def _():
                cwe.wait()
                emb_stage()
                gn_params(1)

            @pl.when(s == 7)
            def _():
                gn_params(2)

            jax.lax.cond((s & 1) == 0, lambda: step(s, 0, True), lambda: step(s, 1, True))
            return carry

        def body2(s, carry):
            @pl.when(s == 11)
            def _():
                gn_params(3)

            jax.lax.cond((s & 1) == 0, lambda: step(s, 0, False), lambda: step(s, 1, False))

            @pl.when(s >= 9)
            def _():
                for g in range(NG):
                    out_copy(s - 1, g).start()
            return carry

        jax.lax.fori_loop(0, 8, body1, 0)
        jax.lax.fori_loop(8, 16, body2, 0)

        last = out_chain(15, m1)
        nper = len(last) // NG
        for g in range(NG):
            run_chains([(0, last[g * nper:(g + 1) * nper])], paced=False)
            out_copy(15, g).start()
        for s in range(8, 16):
            for g in range(NG):
                out_copy(s, g).wait()

    return kernel


_KERNEL = make_kernel({'T': 9700, 'TU': 7000, 'TO1': 8800, 'TI1': 8800})


@jax.jit
def pallas_standalone__adm_resblock__diffusion_kernel(x, t_emb, g1, be1, w1, w_emb, g2, be2, w2):
    xh = jnp.transpose(x, (0, 2, 3, 1))
    w1t = jnp.transpose(w1, (2, 3, 0, 1))
    w2t = jnp.transpose(w2, (2, 3, 0, 1))
    hb = pl.BlockSpec(memory_space=pl.ANY)
    out = pl.pallas_call(
        _KERNEL,
        out_shape=jax.ShapeDtypeStruct((B, H, W, C), BF16),
        in_specs=[hb] * 9,
        out_specs=hb,
        scratch_shapes=[
            pltpu.VMEM((B, EMB), BF16),
            pltpu.VMEM((C,), BF16),
            pltpu.VMEM((C,), BF16),
            pltpu.VMEM((C,), BF16),
            pltpu.VMEM((C,), BF16),
            pltpu.VMEM((2, 3, 3, C // 2, C), U32),
            pltpu.VMEM((EMB, C), BF16),
            pltpu.VMEM((NPOS, C // 2, C), U32),
            pltpu.VMEM((NPOS + 1, C // 2, C), U32),
            pltpu.VMEM((6, H + 1, NG, TW, LG), U32),
            pltpu.VMEM((NPOS + 1, MC // 2, C), U32),
            pltpu.VMEM((NPOS + 1, MC // 2, C), U32),
            pltpu.VMEM((NPOS, MC, C), F32),
            pltpu.VMEM((NPOS, MC, C), F32),
            pltpu.VMEM((2 * NR * 12 + 1, 8, LG), F32),
            pltpu.VMEM((5, NCH, 2, 8, C), F32),
            pltpu.VMEM((4, 1, C), F32),
            pltpu.VMEM((2, 2, 1, C), F32),
            pltpu.VMEM((4, 2, 8, C), F32),
            pltpu.VMEM((8, LG), U32),
            pltpu.SMEM((8,), jnp.int32),
            pltpu.SemaphoreType.DMA((80,)),
        ],
        compiler_params=pltpu.CompilerParams(vmem_limit_bytes=120 * 2 ** 20),
    )(xh, t_emb, g1, be1, w1t, w_emb, g2, be2, w2t)
    return jnp.transpose(out, (0, 3, 1, 2))
```

```python
import functools
import jax
import jax.numpy as jnp
from jax.experimental import pallas as pl
from jax.experimental.pallas import tpu as pltpu

B, C, H, W, EMB = 2, 512, 64, 64, 1152
NG, LG = 4, 128
TH = 4
NP = 6
NPOS = NP * NP
TW = W // 2
CT = 4
MC = CT * (W // TH)
RC = CT * TH
NCH = H // RC
NR = RC + 2
EPS = 1e-5
F32 = jnp.float32
BF16 = jnp.bfloat16
U32 = jnp.uint32

PA, PB = 2.0 / 3.0, 1.5


CA = 1.0 / (2.0 * PA * PA * (PA * PA - PB * PB))
CB = 1.0 / (PA * PA * 2.0 * PB * PB * (PB * PB - PA * PA))


def _bt(d):
    a2, b2 = PA * PA, PB * PB
    d0, d1, d2, d3, d4, d5 = d
    p2 = b2 * d2
    aa = d4 - p2
    ra = PA * (d3 - b2 * d1)
    ab = d4 - a2 * d2
    rb = PB * (d3 - a2 * d1)
    t0 = (d0 + ab) - p2
    t5 = (d1 + d5) - (a2 + b2) * d3
    return [t0, aa + ra, aa - ra, ab + rb, ab - rb, t5]


def _at(m):
    m0, m1, m2, m3, m4, m5 = m
    sa, da = m1 + m2, m1 - m2
    sb, db = m3 + m4, m3 - m4
    y0 = (m0 + CA * sa) + CB * sb
    y1 = (CA * PA) * da + (CB * PB) * db
    y2 = (CA * PA * PA) * sa + (CB * PB * PB) * sb
    y3 = ((CA * PA ** 3) * da + (CB * PB ** 3) * db) + m5
    return [y0, y1, y2, y3]


def _gt(g0, g1, g2):
    a2 = PA * PA
    od = PA * g1
    ea = g0 + a2 * g2
    eb = a2 * g0 + g2
    return [g0, ea + od, ea - od, eb + od, eb - od, g2]


def _unpack(w, idx):
    return pltpu.unpack_elementwise(w, index=idx, packed_dtype=BF16, unpacked_dtype=F32)


def _pack(lo, hi):
    return pltpu.pack_elementwise([lo, hi], packed_dtype=BF16)


def _gs(g):
    return slice(g * LG, (g + 1) * LG)


def _static(s):
    return isinstance(s, int)


def make_kernel(cfg):
    T_IN = cfg.get('TI', cfg.get('T', 9500))
    T_OUT = cfg.get('TO', cfg.get('T', 9500))
    L_R, L_H = cfg.get('L_R', 40), cfg.get('L_H', 22)
    L_A, L_C = cfg.get('L_A', 20), cfg.get('L_C', 26)
    L_U, T_U, URB = cfg.get('L_U', 30), cfg.get('TU', cfg.get('T', 9500)), cfg.get('URB', 5)
    NRB = 2

    def kernel(x_hbm, t_hbm, g1_hbm, be1_hbm, w1_hbm, wemb_hbm, g2_hbm, be2_hbm, w2_hbm,
               out_hbm,
               t_ref, g1_ref, be1_ref, g2_ref, be2_ref,
               wraw, wembs, ua, ub, uc, ud, u2_ref, src, v0, v1, m0, m1, me, rbuf, stats, embtab, gbt, gnp, zvr, zsm, sems):
        vbuf = (v0, v1)
        u1g = (ua, ub, uc, ud)
        mbuf = (m0, m1)
        xb = x_hbm.bitcast(U32)
        ob_ = out_hbm.bitcast(U32)
        w1b = w1_hbm.bitcast(U32)
        w2b = w2_hbm.bitcast(U32)

        def delay(tok_u32, cyc):
            t = pltpu.bitcast(tok_u32, F32)
            n, rem = divmod(cyc, 116)
            for _ in range(n):
                t = jnp.broadcast_to(jnp.sum(t, axis=1, keepdims=True), (8, LG))
            for _ in range(rem // 8):
                t = jnp.tanh(t)
            return t

        def run_chains(chains, paced=True):
            items = []
            for ci, (tt, ch) in enumerate(chains):
                n = len(ch)
                nat = sum(c[1] for c in ch)
                extra = max(0.0, (tt - nat) / n)
                for k, (fn, lat) in enumerate(ch):
                    items.append(((k + 0.5) / n, ci, fn, int(extra)))
            items.sort(key=lambda it: (it[0], it[1]))
            toks = [None] * len(chains)
            for _, ci, fn, d in items:
                raw = fn(toks[ci])
                toks[ci] = delay(raw, d) if paced else None

        def anchor(vals):
            b = [pltpu.bitcast(v, U32) for v in vals]
            while len(b) > 1:
                b = [b[i] | b[i + 1] if i + 1 < len(b) else b[i] for i in range(0, len(b), 2)]
            return b[0] & zvr[...]

        def inj(x, tok):
            return x if tok is None else x + tok

        def x_stats(img, row0, nrows, slot):
            for g in range(NG):
                a1 = [jnp.zeros((8, LG), F32)] * 2
                a2 = [jnp.zeros((8, LG), F32)] * 2
                for j in range(nrows):
                    for t in range(TW // 8):
                        w = src[img, row0 + j, g, pl.ds(8 * t, 8), :]
                        e, o = _unpack(w, 0), _unpack(w, 1)
                        a1[t % 2] = a1[t % 2] + (e + o)
                        a2[t % 2] = a2[t % 2] + (e * e + o * o)
                stats[img, slot, 0, :, _gs(g)] = a1[0] + a1[1]
                stats[img, slot, 1, :, _gs(g)] = a2[0] + a2[1]

        def w_unit(tok, g, ob, cb):
            raw = [[[None] * 3 for _ in range(3)] for _ in range(2)]
            for i in range(3):
                for j in range(3):
                    w = wraw[0, i, j, pl.ds(g * (LG // 2) + ob, 8), _gs(cb)]
                    raw[0][i][j], raw[1][i][j] = _unpack(w, 0), _unpack(w, 1)
            raw[0][0][1] = inj(raw[0][0][1], tok)
            wq = [[_gt(*raw[par][i]) for i in range(3)] for par in range(2)]
            for q in range(NP):
                o0 = _gt(*[wq[0][i][q] for i in range(3)])
                o1 = _gt(*[wq[1][i][q] for i in range(3)])
                for p in range(NP):
                    u1g[g][p * NP + q, pl.ds(ob, 8), _gs(cb)] = _pack(o0[p], o1[p])
            if cfg.get('wtok', 0) == 1:
                return anchor([o0[1], o1[1]])
            return u1g[g][zsm[0], 0:8, 0:LG]

        def u_chain(conv, dst, obs):
            a2 = PA * PA
            units = []
            for ob in obs:
                for cb in range(NG):
                    def u_link(tok, ob=ob, cb=cb, qs=()):
                        js = (0,) if qs == (0,) else (2,) if qs == (5,) else (0, 1, 2)
                        wq = [[], []]
                        for i in range(3):
                            w = [wraw[conv, i, j, pl.ds(ob, 8), _gs(cb)] for j in js]
                            for par in range(2):
                                r = [_unpack(x, par) for x in w]
                                if par == 0:
                                    r[0] = inj(r[0], tok)
                                if len(js) == 1:
                                    wq[par].append(r)
                                else:
                                    od = PA * r[1]
                                    ev = r[0] + a2 * r[2] if qs == (1, 2) else a2 * r[0] + r[2]
                                    wq[par].append([ev + od, ev - od])
                        for qi, q in enumerate(qs):
                            o0 = _gt(*[wq[0][i][qi] for i in range(3)])
                            o1 = _gt(*[wq[1][i][qi] for i in range(3)])
                            for p in range(NP):
                                dst[p * NP + q, pl.ds(ob, 8), _gs(cb)] = _pack(o0[p], o1[p])
                        return dst[zsm[0], 0:8, 0:LG]

                    units.append((functools.partial(u_link, qs=(0,)), L_U // 2))
                    units.append((functools.partial(u_link, qs=(1, 2)), L_U))
                    units.append((functools.partial(u_link, qs=(3, 4)), L_U))
                    units.append((functools.partial(u_link, qs=(5,)), L_U // 2))
            return units

        def emb_stage():
            t = t_ref[...].astype(F32)
            st = (t * jax.nn.sigmoid(t)).astype(BF16)
            emb = jnp.dot(st, wembs[...], preferred_element_type=F32)
            embtab[2] = emb[0:1]
            embtab[3] = emb[1:2]

        def gn_params(sidx):
            conv = sidx >> 1
            s1 = stats[sidx, 0, 0] + stats[sidx, 1, 0] + stats[sidx, 2, 0] + stats[sidx, 3, 0]
            s2 = stats[sidx, 0, 1] + stats[sidx, 1, 1] + stats[sidx, 2, 1] + stats[sidx, 3, 1]
            s1 = jnp.sum(s1, axis=0, keepdims=True)
            s2 = jnp.sum(s2, axis=0, keepdims=True)
            e = embtab[sidx]
            n = float(H * W)
            t1 = s1 + n * e
            t2 = s2 + (2.0 * e) * s1 + (n * e) * e
            gam = gbt[conv, 0]
            bet = gbt[conv, 1]
            inv = 1.0 / (H * W * LG)
            for g in range(NG):
                mean = jnp.sum(t1[:, _gs(g)], axis=1, keepdims=True) * inv
                ex2 = jnp.sum(t2[:, _gs(g)], axis=1, keepdims=True) * inv
                var = jnp.maximum(ex2 - mean * mean, 0.0)
                rstd = jax.lax.rsqrt(var + EPS)
                sc = gam[:, _gs(g)] * rstd
                sh = bet[:, _gs(g)] + (e[:, _gs(g)] - mean) * sc
                gnp[sidx, 0, :, _gs(g)] = jnp.broadcast_to(0.5 * sc, (8, LG))
                gnp[sidx, 1, :, _gs(g)] = jnp.broadcast_to(0.5 * sh, (8, LG))

        def in_chain(s, vdst, edge):
            sidx = s >> 2
            chunk = s & 3
            r0 = chunk * RC - 1
            sub = jax.lax.broadcasted_iota(jnp.int32, (8, LG), 0)
            units = []
            for g in range(NG):
                base = (g % NRB) * NR * 12

                def row_link(tok, g=g, base=base, lr=0):
                    r = r0 + lr
                    valid = None
                    zero_row = False
                    if _static(r):
                        zero_row = r < 0 or r >= H
                    elif lr == 0 and edge in ('top', 'both'):
                        valid = r >= 0
                        r = jnp.maximum(r, 0)
                    elif lr == NR - 1 and edge in ('bot', 'both'):
                        valid = r < H
                        r = jnp.minimum(r, H - 1)
                    if zero_row:
                        z = jnp.zeros((8, LG), F32)
                        for q in range(12):
                            rbuf[base + lr * 12 + q] = z
                    else:
                        sc = inj(gnp[sidx, 0, :, _gs(g)], tok)
                        sh = gnp[sidx, 1, :, _gs(g)]
                        c = []
                        for j in range(4):
                            w = src[sidx, r, g, pl.ds(j, 8, stride=4), :]
                            for half in range(2):
                                hv = _unpack(w, half) * sc + sh
                                a = hv + hv * jnp.tanh(hv)
                                if valid is not None:
                                    a = jnp.where(valid, a, 0.0)
                                c.append(a)
                        left = jnp.where(sub == 0, 0.0, pltpu.roll(c[7], 1, 0))
                        right = jnp.where(sub == 7, 0.0, pltpu.roll(c[0], 7, 0))
                        ev = _bt([left, c[0], c[1], c[2], c[3], c[4]])
                        od = _bt([c[3], c[4], c[5], c[6], c[7], right])
                        for q in range(NP):
                            rbuf[base + lr * 12 + q] = ev[q]
                            rbuf[base + lr * 12 + 6 + q] = od[q]
                    return pltpu.bitcast(rbuf[zsm[2]], U32)

                def col_link(tok, g=g, base=base, ty=0, q=0):
                    t = []
                    for par in range(2):
                        d = [rbuf[base + (ty * TH + i) * 12 + 6 * par + q] for i in range(NP)]
                        if par == 0:
                            d[2] = inj(d[2], tok)
                        t.append(_bt(d))
                    for p in range(NP):
                        vdst[p * NP + q, pl.ds(ty * 8, 8), _gs(g)] = _pack(t[0][p], t[1][p])
                    return vdst[zsm[0], 0:8, 0:LG]

                for ty in range(CT):
                    for lr in range(0 if ty == 0 else ty * TH + 2, ty * TH + NP):
                        units.append((functools.partial(row_link, lr=lr), L_R))
                    for q in range(NP):
                        units.append((functools.partial(col_link, ty=ty, q=q), L_H))
            return units

        def out_chain(s, msrc, conv1=False):
            img = (s >> 2) & 1
            chunk = s & 3
            kind2 = False if conv1 else s >= 8
            if conv1:
                dslot, sslot, rslot = 2 + img, 2 + img, 0
            elif _static(s):
                dslot = (4 if kind2 else 2) + img
                sslot = 4 if kind2 else 2 + img
                rslot = img if kind2 else 0
            else:
                dslot = jnp.where(kind2, 4, 2) + img
                sslot = jnp.where(kind2, 4, 2 + img)
                rslot = jnp.where(kind2, img, 0)
            need_stats = not (_static(s) and kind2)
            units = []
            for g in range(NG):
                acc = [jnp.zeros((8, LG), F32), jnp.zeros((8, LG), F32)]
                for b in range(2 * CT):
                    hold = {}

                    def w_link(tok, g=g, b=b, hold=hold, ps=()):
                        vals = []
                        for p in ps:
                            mref, lanes = msrc[g] if isinstance(msrc, dict) else (msrc, _gs(g))
                            mm = [mref[p * NP + q, pl.ds(8 * b, 8), lanes] for q in range(NP)]
                            if p == ps[0]:
                                mm[1] = inj(mm[1], tok)
                            hold[p] = _at(mm)
                            vals += hold[p]
                        return anchor(vals)

                    def fin_link(tok, g=g, b=b, acc=acc, hold=hold, e=0):
                        ty, hh = b // 2, b % 2
                        xw = []
                        for k in range(0 if conv1 else TH):
                            r = chunk * RC + ty * TH + k
                            if _static(s):
                                rr = r if kind2 else H
                            else:
                                rr = jnp.where(kind2, r, H)
                            xw.append(src[rslot, rr, g, pl.ds(16 * hh + e, 8, stride=2), :])
                        y = []
                        for l in (2 * e, 2 * e + 1):
                            col = [hold[p][l] for p in range(NP)]
                            col[1] = inj(col[1], tok)
                            y.append(_at(col))
                        for k in range(TH):
                            r = chunk * RC + ty * TH + k
                            ye, yo = y[0][k], y[1][k]
                            if need_stats:
                                acc[0] = acc[0] + (ye + yo)
                                acc[1] = acc[1] + (ye * ye + yo * yo)
                            if not conv1:
                                ye, yo = ye + _unpack(xw[k], 0), yo + _unpack(xw[k], 1)
                            src[dslot, r, g, pl.ds(16 * hh + e, 8, stride=2), :] = _pack(ye, yo)
                        if need_stats and b == 2 * CT - 1 and e == 1:
                            stats[sslot, chunk, 0, :, _gs(g)] = acc[0]
                            stats[sslot, chunk, 1, :, _gs(g)] = acc[1]
                        tk = src[0, zsm[1], 0, 0:8, :]
                        if need_stats:
                            tk = tk | anchor(acc)
                        return tk

                    units.append((functools.partial(w_link, ps=(0, 1, 2)), L_A))
                    units.append((functools.partial(w_link, ps=(3, 4, 5)), L_A))
                    units.append((functools.partial(fin_link, e=0), L_C))
                    units.append((functools.partial(fin_link, e=1), L_C))
            return units

        def stage_mm(vsrc, mdst, conv1):
            for pos in range(NPOS):
                v = pltpu.bitcast(vsrc[pos], BF16)
                for g in range(NG):
                    u = u1g[g][pos] if conv1 else u2_ref[pos, pl.ds(g * (LG // 2), LG // 2), :]
                    mdst[pos, :, _gs(g)] = jax.lax.dot_general(v, pltpu.bitcast(u, BF16), (((1,), (1,)), ((), ())),
                                                               preferred_element_type=F32)

        def stage_mm_g(vsrc, mdst, lanes, usrc, row0):
            for pos in range(NPOS):
                v = pltpu.bitcast(vsrc[pos], BF16)
                u = pltpu.bitcast(usrc[pos, pl.ds(row0, LG // 2), :], BF16)
                mdst[pos, :, lanes] = jax.lax.dot_general(v, u, (((1,), (1,)), ((), ())),
                                                          preferred_element_type=F32)

        def out_copy(s, g):
            img = (s >> 2) & 1
            chunk = s & 3
            return pltpu.make_async_copy(src.at[4 + img, pl.ds(chunk * RC, RC), g],
                                         ob_.at[img, pl.ds(chunk * RC, RC), :, pl.ds(g * LG, LG)],
                                         sems.at[48 + (s - 8) * NG + g])

        def x_copy(img, c, g, nrows, sem):
            return pltpu.make_async_copy(xb.at[img, pl.ds(c * nrows, nrows), :, pl.ds(g * LG, LG)],
                                         src.at[img, pl.ds(c * nrows, nrows), g], sems.at[sem])

        NW1 = cfg.get('NW1', 16)
        WR = (C // 2) // NW1

        def w1_copy(k):
            return pltpu.make_async_copy(w1b.at[:, :, pl.ds(k * WR, WR)],
                                         wraw.at[0, :, :, pl.ds(k * WR, WR)], sems.at[16 + k])

        for c in range(NCH):
            for g in range(NG):
                x_copy(0, c, g, RC, c * NG + g).start()
        small = [pltpu.make_async_copy(a, b, sems.at[40 + i]) for i, (a, b) in enumerate(
            ((g1_hbm, g1_ref), (be1_hbm, be1_ref), (g2_hbm, g2_ref), (be2_hbm, be2_ref), (t_hbm, t_ref)))]
        for cp in small:
            cp.start()
        for k in range(NW1 if cfg.get('dmaonly') != 1 else 0):
            w1_copy(k).start()
        cx1 = [x_copy(1, 0, g, H, 32 + g) for g in range(NG)]
        cwe = pltpu.make_async_copy(wemb_hbm, wembs, sems.at[36])
        cw2 = pltpu.make_async_copy(w2b, wraw.at[1], sems.at[37])
        nod2 = cfg.get('nod2')
        if not nod2:
            cw2.start()
            for cp in cx1:
                cp.start()
            cwe.start()

        zsm[0] = NPOS
        zsm[1] = H
        zsm[2] = NRB * NR * 12
        zsm[3] = 0
        zvr[...] = jnp.zeros((8, LG), U32)
        rbuf[NRB * NR * 12] = jnp.zeros((8, LG), F32)
        v0[NPOS] = jnp.zeros((MC // 2, C), U32)
        v1[NPOS] = jnp.zeros((MC // 2, C), U32)
        u2_ref[NPOS, 0:8, 0:LG] = jnp.zeros((8, LG), U32)
        for g in range(NG):
            u1g[g][NPOS, 0:8, 0:LG] = jnp.zeros((8, LG), U32)
        zsm[3] = 0
        src[0, H] = jnp.zeros((NG, TW, LG), U32)
        zero = jnp.zeros((1, C), F32)
        embtab[0] = zero
        embtab[1] = zero

        if cfg.get('dum'):
            @pl.when(zsm[3] == 1)
            def _():
                for pos in range(cfg['dum']):
                    u_ref[pos] = jnp.full((C // 2, C), pos + 1, U32)

        def xs_body(c, carry):
            for g in range(NG):
                x_copy(0, c, g, RC, c * NG + g).wait()
            x_stats(0, c * RC, RC, c)
            return carry

        def wt_body(k, carry):
            w1_copy(k).wait()
            for kk in range(WR // 8):
                for cb in range(NG):
                    w_unit(None, 0, pl.multiple_of(k * WR + kk * 8, 8), cb)
            return carry

        def prologue():
            if cfg.get('dmaonly'):
                for c in range(NCH):
                    for g in range(NG):
                        x_copy(0, c, g, RC, c * NG + g).wait()
                for cp in small:
                    cp.wait()
                if cfg['dmaonly'] == 2:
                    for k in range(NW1):
                        w1_copy(k).wait()
                return
            jax.lax.fori_loop(0, NCH, xs_body, 0)
            for cp in small:
                cp.wait()
            gbt[0, 0] = g1_ref[...].astype(F32).reshape(1, C)
            gbt[0, 1] = be1_ref[...].astype(F32).reshape(1, C)
            gbt[1, 0] = g2_ref[...].astype(F32).reshape(1, C)
            gbt[1, 1] = be2_ref[...].astype(F32).reshape(1, C)
            gn_params(0)
            run_chains([(0, in_chain(0, v0, None))], paced=False)
            jax.lax.fori_loop(0, NW1 // NG, wt_body, 0)
            in1 = in_chain(1, v1, None)

            nper = len(in1) // NG

            def sub_block(g):
                chs = [(cfg.get('TI0', 2200) if g + 1 < NG else cfg.get('TI3', 2000), in1[g * nper:(g + 1) * nper])]
                if g + 1 < NG:
                    for k in range((g + 1) * NW1 // NG, (g + 2) * NW1 // NG):
                        w1_copy(k).wait()
                    chs.append((cfg.get('TU0', 2200), [(functools.partial(w_unit, g=g + 1, ob=8 * kk, cb=cb), cfg.get('L_W', 60))
                                                       for kk in range(8) for cb in range(NG)]))
                run_chains(chs, paced=not cfg.get('unp0'))
                stage_mm_g(v0, m0, _gs(g), u1g[g], 0)

            def sub_body(i, carry):
                for g in range(NG):
                    pl.when(i == g)(functools.partial(sub_block, g))
                return carry
            jax.lax.fori_loop(0, NG, sub_body, 0)

        if not cfg.get('pin'):
            prologue()

        def step(s, par, conv1):
            cur, nxt = par, 1 - par
            t_out, t_in = (cfg.get('TO1', T_OUT), cfg.get('TI1', T_IN)) if conv1 else (T_OUT, T_IN)
            chs = [(t_out, out_chain(s - 1, mbuf[nxt], conv1)),
                   (t_in, in_chain(jnp.minimum(s + 1, 15), vbuf[nxt], 'top' if par == 1 else 'bot'))]
            if conv1:
                obs = [pl.multiple_of(jnp.minimum((s - 1) * URB + kk, C // 16 - 1) * 8, 8) for kk in range(URB)]
                chs.append((T_U, u_chain(1, u2_ref, obs)))
            run_chains(chs)
            stage_mm(vbuf[cur], mbuf[cur], conv1)

        def body1(s, carry):
            @pl.when(s == 1)
            def _():
                cw2.wait()

            @pl.when(s == 2)
            def _():
                for cp in cx1:
                    cp.wait()

                def xs1(c, cc):
                    x_stats(1, c * RC, RC, c)
                    return cc
                jax.lax.fori_loop(0, NCH, xs1, 0)

            @pl.when(s == 3)
            def _():
                cwe.wait()
                emb_stage()
                gn_params(1)

            @pl.when(s == 7)
            def _():
                gn_params(2)

            jax.lax.cond((s & 1) == 0, lambda: step(s, 0, True), lambda: step(s, 1, True))
            return carry

        mlast = {g: ((m1, _gs(g)) if g % 2 == 0 else (me, slice(0, LG))) for g in range(NG)}
        o14 = out_chain(14, m0)
        o15 = out_chain(15, mlast)
        nper = len(o15) // NG

        def last_block(g):
            g14 = (2 * g, 2 * g + 1) if g < 2 else ()
            chs = []
            if g14:
                chs.append((cfg.get('TL', 2000), o14[g14[0] * nper:(g14[1] + 1) * nper]))
            if g > 0:
                chs.append((cfg.get('TL', 2000), o15[(g - 1) * nper:g * nper]))
            run_chains(chs)
            stage_mm_g(v1, mlast[g][0], mlast[g][1], u2_ref, g * (LG // 2))
            for gg in g14:
                out_copy(14, gg).start()
            if g > 0:
                out_copy(15, g - 1).start()

        def last_body(i, carry):
            for g in range(NG):
                pl.when(i == g)(functools.partial(last_block, g))
            return carry

        def body2(s, carry):
            @pl.when(s == 11)
            def _():
                gn_params(3)

            jax.lax.cond((s & 1) == 0, lambda: step(s, 0, False), lambda: step(s, 1, False))

            @pl.when(s >= 9)
            def _():
                for g in range(NG):
                    out_copy(s - 1, g).start()
            return carry

        jax.lax.fori_loop(1, 8, body1, 0)

        if cfg.get('lastsplit'):
            jax.lax.fori_loop(8, 15, body2, 0)
            jax.lax.fori_loop(0, NG, last_body, 0)
            run_chains([(0, o15[(NG - 1) * nper:])], paced=False)
            out_copy(15, NG - 1).start()
        else:
            jax.lax.fori_loop(8, 16, body2, 0)
            last = out_chain(15, m1)
            for g in range(NG):
                run_chains([(0, last[g * nper:(g + 1) * nper])], paced=False)
                out_copy(15, g).start()
        for s in range(8, 16):
            for g in range(NG):
                out_copy(s, g).wait()

    return kernel


_KERNEL = make_kernel({'T': 9700, 'TU': 7000, 'TO1': 8800, 'TI1': 8800, 'TU0': 2800, 'TI0': 2800, 'wtok': 1})


@jax.jit
def pallas_standalone__adm_resblock__diffusion_kernel(x, t_emb, g1, be1, w1, w_emb, g2, be2, w2):
    xh = jnp.transpose(x, (0, 2, 3, 1))
    w1t = jnp.transpose(w1, (2, 3, 0, 1))
    w2t = jnp.transpose(w2, (2, 3, 0, 1))
    hb = pl.BlockSpec(memory_space=pl.ANY)
    out = pl.pallas_call(
        _KERNEL,
        out_shape=jax.ShapeDtypeStruct((B, H, W, C), BF16),
        in_specs=[hb] * 9,
        out_specs=hb,
        scratch_shapes=[
            pltpu.VMEM((B, EMB), BF16),
            pltpu.VMEM((C,), BF16),
            pltpu.VMEM((C,), BF16),
            pltpu.VMEM((C,), BF16),
            pltpu.VMEM((C,), BF16),
            pltpu.VMEM((2, 3, 3, C // 2, C), U32),
            pltpu.VMEM((EMB, C), BF16),
            pltpu.VMEM((NPOS + 1, LG // 2, C), U32),
            pltpu.VMEM((NPOS + 1, LG // 2, C), U32),
            pltpu.VMEM((NPOS + 1, LG // 2, C), U32),
            pltpu.VMEM((NPOS + 1, LG // 2, C), U32),
            pltpu.VMEM((NPOS + 1, C // 2, C), U32),
            pltpu.VMEM((6, H + 1, NG, TW, LG), U32),
            pltpu.VMEM((NPOS + 1, MC // 2, C), U32),
            pltpu.VMEM((NPOS + 1, MC // 2, C), U32),
            pltpu.VMEM((NPOS, MC, C), F32),
            pltpu.VMEM((NPOS, MC, C), F32),
            pltpu.VMEM((NPOS, MC, LG), F32),
            pltpu.VMEM((2 * NR * 12 + 1, 8, LG), F32),
            pltpu.VMEM((5, NCH, 2, 8, C), F32),
            pltpu.VMEM((4, 1, C), F32),
            pltpu.VMEM((2, 2, 1, C), F32),
            pltpu.VMEM((4, 2, 8, C), F32),
            pltpu.VMEM((8, LG), U32),
            pltpu.SMEM((8,), jnp.int32),
            pltpu.SemaphoreType.DMA((88,)),
        ],
        compiler_params=pltpu.CompilerParams(vmem_limit_bytes=120 * 2 ** 20),
    )(xh, t_emb, g1, be1, w1t, w_emb, g2, be2, w2t)
    return jnp.transpose(out, (0, 3, 1, 2))
```

```python
import functools
import jax
import jax.numpy as jnp
from jax.experimental import pallas as pl
from jax.experimental.pallas import tpu as pltpu

B, C, H, W, EMB = 2, 512, 64, 64, 1152
NG, LG = 4, 128
TH = 4
NP = 6
NPOS = NP * NP
TW = W // 2
CT = 4
MC = CT * (W // TH)
RC = CT * TH
NCH = H // RC
NR = RC + 2
EPS = 1e-5
F32 = jnp.float32
BF16 = jnp.bfloat16
U32 = jnp.uint32

PA, PB = 2.0 / 3.0, 1.5


CA = 1.0 / (2.0 * PA * PA * (PA * PA - PB * PB))
CB = 1.0 / (PA * PA * 2.0 * PB * PB * (PB * PB - PA * PA))


def _bt(d):
    a2, b2 = PA * PA, PB * PB
    d0, d1, d2, d3, d4, d5 = d
    p2 = b2 * d2
    aa = d4 - p2
    ra = PA * (d3 - b2 * d1)
    ab = d4 - a2 * d2
    rb = PB * (d3 - a2 * d1)
    t0 = (d0 + ab) - p2
    t5 = (d1 + d5) - (a2 + b2) * d3
    return [t0, aa + ra, aa - ra, ab + rb, ab - rb, t5]


def _at(m):
    m0, m1, m2, m3, m4, m5 = m
    sa, da = m1 + m2, m1 - m2
    sb, db = m3 + m4, m3 - m4
    y0 = (m0 + CA * sa) + CB * sb
    y1 = (CA * PA) * da + (CB * PB) * db
    y2 = (CA * PA * PA) * sa + (CB * PB * PB) * sb
    y3 = ((CA * PA ** 3) * da + (CB * PB ** 3) * db) + m5
    return [y0, y1, y2, y3]


def _gt(g0, g1, g2):
    a2 = PA * PA
    od = PA * g1
    ea = g0 + a2 * g2
    eb = a2 * g0 + g2
    return [g0, ea + od, ea - od, eb + od, eb - od, g2]


def _unpack(w, idx):
    return pltpu.unpack_elementwise(w, index=idx, packed_dtype=BF16, unpacked_dtype=F32)


def _pack(lo, hi):
    return pltpu.pack_elementwise([lo, hi], packed_dtype=BF16)


def _gs(g):
    return slice(g * LG, (g + 1) * LG)


def _static(s):
    return isinstance(s, int)


def make_kernel(cfg):
    T2 = cfg.get('T2', 9700)
    T1 = cfg.get('T1', 8800)
    T_U = cfg.get('TU', 7000)
    T0, T0L = cfg.get('T0', 2600), cfg.get('T0L', 2500)
    ISP = cfg.get('isp', [0, 36, 72, 108, 168])
    L_R, L_H, L_A, L_C, L_U, L_W = 40, 22, 20, 26, 30, 60
    URB = 5
    NRB = 2

    def kernel(x_hbm, t_hbm, g1_hbm, be1_hbm, w1_hbm, wemb_hbm, g2_hbm, be2_hbm, w2_hbm,
               out_hbm,
               t_ref, g1_ref, be1_ref, g2_ref, be2_ref,
               wraw, wembs, ua, ub, uc, ud, u2_ref, src, v0, v1, m0, m1, rbuf, stats, embtab, gbt, gnp, zvr, zsm, sems):
        vbuf = (v0, v1)
        u1g = (ua, ub, uc, ud)
        mbuf = (m0, m1)
        xb = x_hbm.bitcast(U32)
        ob_ = out_hbm.bitcast(U32)
        w1b = w1_hbm.bitcast(U32)
        w2b = w2_hbm.bitcast(U32)

        def delay(tok_u32, cyc):
            t = pltpu.bitcast(tok_u32, F32)
            n, rem = divmod(cyc, 116)
            for _ in range(n):
                t = jnp.broadcast_to(jnp.sum(t, axis=1, keepdims=True), (8, LG))
            for _ in range(rem // 8):
                t = jnp.tanh(t)
            return t

        def run_chains(chains, paced=True):
            items = []
            for ci, (tt, ch) in enumerate(chains):
                n = len(ch)
                nat = sum(c[1] for c in ch)
                extra = max(0.0, (tt - nat) / n)
                for k, (fn, lat) in enumerate(ch):
                    items.append(((k + 0.5) / n, ci, fn, int(extra)))
            items.sort(key=lambda it: (it[0], it[1]))
            toks = [None] * len(chains)
            for _, ci, fn, d in items:
                raw = fn(toks[ci])
                toks[ci] = delay(raw, d) if paced else None

        def anchor(vals):
            b = [pltpu.bitcast(v, U32) for v in vals]
            while len(b) > 1:
                b = [b[i] | b[i + 1] if i + 1 < len(b) else b[i] for i in range(0, len(b), 2)]
            return b[0] & zvr[...]

        def inj(x, tok):
            return x if tok is None else x + tok

        def x_stats(img, row0, nrows, slot, groups=range(NG)):
            for g in groups:
                a1 = [jnp.zeros((8, LG), F32)] * 2
                a2 = [jnp.zeros((8, LG), F32)] * 2
                for j in range(nrows):
                    for t in range(TW // 8):
                        w = src[img, row0 + j, g, pl.ds(8 * t, 8), :]
                        e, o = _unpack(w, 0), _unpack(w, 1)
                        a1[t % 2] = a1[t % 2] + (e + o)
                        a2[t % 2] = a2[t % 2] + (e * e + o * o)
                stats[img, slot, 0, :, _gs(g)] = a1[0] + a1[1]
                stats[img, slot, 1, :, _gs(g)] = a2[0] + a2[1]

        def x1_chain(groups):
            units = []
            for g in groups:
                for c in range(NCH):
                    acc = [jnp.zeros((8, LG), F32), jnp.zeros((8, LG), F32)]

                    def s_link(tok, g=g, c=c, acc=acc, j0=0):
                        for j in range(j0, j0 + 4):
                            for t in range(TW // 8):
                                w = src[1, c * RC + j, g, pl.ds(8 * t, 8), :]
                                e, o = _unpack(w, 0), _unpack(w, 1)
                                if t % 2 == 0:
                                    e = inj(e, tok)
                                acc[0] = acc[0] + (e + o)
                                acc[1] = acc[1] + (e * e + o * o)
                        if j0 + 4 == RC:
                            stats[1, c, 0, :, _gs(g)] = acc[0]
                            stats[1, c, 1, :, _gs(g)] = acc[1]
                        return anchor(acc)

                    for j0 in range(0, RC, 4):
                        units.append((functools.partial(s_link, j0=j0), 40))
            return units

        def w_unit(tok, g, ob, cb):
            raw = [[[None] * 3 for _ in range(3)] for _ in range(2)]
            for i in range(3):
                for j in range(3):
                    w = wraw[0, i, j, pl.ds(g * (LG // 2) + ob, 8), _gs(cb)]
                    raw[0][i][j], raw[1][i][j] = _unpack(w, 0), _unpack(w, 1)
            raw[0][0][1] = inj(raw[0][0][1], tok)
            wq = [[_gt(*raw[par][i]) for i in range(3)] for par in range(2)]
            for q in range(NP):
                o0 = _gt(*[wq[0][i][q] for i in range(3)])
                o1 = _gt(*[wq[1][i][q] for i in range(3)])
                for p in range(NP):
                    u1g[g][p * NP + q, pl.ds(ob, 8), _gs(cb)] = _pack(o0[p], o1[p])
            return anchor([o0[1], o1[1]])

        def u_chain(obs):
            a2 = PA * PA
            units = []
            for ob in obs:
                for cb in range(NG):
                    def u_link(tok, ob=ob, cb=cb, qs=()):
                        js = (0,) if qs == (0,) else (2,) if qs == (5,) else (0, 1, 2)
                        wq = [[], []]
                        for i in range(3):
                            w = [wraw[1, i, j, pl.ds(ob, 8), _gs(cb)] for j in js]
                            for par in range(2):
                                r = [_unpack(x, par) for x in w]
                                if par == 0:
                                    r[0] = inj(r[0], tok)
                                if len(js) == 1:
                                    wq[par].append(r)
                                else:
                                    od = PA * r[1]
                                    ev = r[0] + a2 * r[2] if qs == (1, 2) else a2 * r[0] + r[2]
                                    wq[par].append([ev + od, ev - od])
                        for qi, q in enumerate(qs):
                            o0 = _gt(*[wq[0][i][qi] for i in range(3)])
                            o1 = _gt(*[wq[1][i][qi] for i in range(3)])
                            for p in range(NP):
                                u2_ref[p * NP + q, pl.ds(ob, 8), _gs(cb)] = _pack(o0[p], o1[p])
                        return u2_ref[zsm[0], 0:8, 0:LG]

                    units.append((functools.partial(u_link, qs=(0,)), L_U // 2))
                    units.append((functools.partial(u_link, qs=(1, 2)), L_U))
                    units.append((functools.partial(u_link, qs=(3, 4)), L_U))
                    units.append((functools.partial(u_link, qs=(5,)), L_U // 2))
            return units

        def emb_stage():
            t = t_ref[...].astype(F32)
            st = (t * jax.nn.sigmoid(t)).astype(BF16)
            emb = jnp.dot(st, wembs[...], preferred_element_type=F32)
            embtab[2] = emb[0:1]
            embtab[3] = emb[1:2]

        def gn_params(sidx):
            conv = sidx >> 1
            s1 = stats[sidx, 0, 0] + stats[sidx, 1, 0] + stats[sidx, 2, 0] + stats[sidx, 3, 0]
            s2 = stats[sidx, 0, 1] + stats[sidx, 1, 1] + stats[sidx, 2, 1] + stats[sidx, 3, 1]
            s1 = jnp.sum(s1, axis=0, keepdims=True)
            s2 = jnp.sum(s2, axis=0, keepdims=True)
            e = embtab[sidx]
            n = float(H * W)
            t1 = s1 + n * e
            t2 = s2 + (2.0 * e) * s1 + (n * e) * e
            gam = gbt[conv, 0]
            bet = gbt[conv, 1]
            inv = 1.0 / (H * W * LG)
            for g in range(NG):
                mean = jnp.sum(t1[:, _gs(g)], axis=1, keepdims=True) * inv
                ex2 = jnp.sum(t2[:, _gs(g)], axis=1, keepdims=True) * inv
                var = jnp.maximum(ex2 - mean * mean, 0.0)
                rstd = jax.lax.rsqrt(var + EPS)
                sc = gam[:, _gs(g)] * rstd
                sh = bet[:, _gs(g)] + (e[:, _gs(g)] - mean) * sc
                gnp[sidx, 0, :, _gs(g)] = jnp.broadcast_to(0.5 * sc, (8, LG))
                gnp[sidx, 1, :, _gs(g)] = jnp.broadcast_to(0.5 * sh, (8, LG))

        def in_chain(s, vdst, edge):
            sidx = s >> 2
            chunk = s & 3
            r0 = chunk * RC - 1
            sub = jax.lax.broadcasted_iota(jnp.int32, (8, LG), 0)
            units = []
            for g in range(NG):
                base = (g % NRB) * NR * 12

                def row_link(tok, g=g, base=base, lr=0):
                    r = r0 + lr
                    valid = None
                    zero_row = False
                    if _static(r):
                        zero_row = r < 0 or r >= H
                    elif lr == 0 and edge in ('top', 'both'):
                        valid = r >= 0
                        r = jnp.maximum(r, 0)
                    elif lr == NR - 1 and edge in ('bot', 'both'):
                        valid = r < H
                        r = jnp.minimum(r, H - 1)
                    if zero_row:
                        z = jnp.zeros((8, LG), F32)
                        for q in range(12):
                            rbuf[base + lr * 12 + q] = z
                    else:
                        sc = inj(gnp[sidx, 0, :, _gs(g)], tok)
                        sh = gnp[sidx, 1, :, _gs(g)]
                        c = []
                        for j in range(4):
                            w = src[sidx, r, g, pl.ds(j, 8, stride=4), :]
                            for half in range(2):
                                hv = _unpack(w, half) * sc + sh
                                a = hv + hv * jnp.tanh(hv)
                                if valid is not None:
                                    a = jnp.where(valid, a, 0.0)
                                c.append(a)
                        left = jnp.where(sub == 0, 0.0, pltpu.roll(c[7], 1, 0))
                        right = jnp.where(sub == 7, 0.0, pltpu.roll(c[0], 7, 0))
                        ev = _bt([left, c[0], c[1], c[2], c[3], c[4]])
                        od = _bt([c[3], c[4], c[5], c[6], c[7], right])
                        for q in range(NP):
                            rbuf[base + lr * 12 + q] = ev[q]
                            rbuf[base + lr * 12 + 6 + q] = od[q]
                    return pltpu.bitcast(rbuf[zsm[2]], U32)

                def col_link(tok, g=g, base=base, ty=0, q=0):
                    t = []
                    for par in range(2):
                        d = [rbuf[base + (ty * TH + i) * 12 + 6 * par + q] for i in range(NP)]
                        if par == 0:
                            d[2] = inj(d[2], tok)
                        t.append(_bt(d))
                    for p in range(NP):
                        vdst[p * NP + q, pl.ds(ty * 8, 8), _gs(g)] = _pack(t[0][p], t[1][p])
                    return vdst[zsm[0], 0:8, 0:LG]

                for ty in range(CT):
                    for lr in range(0 if ty == 0 else ty * TH + 2, ty * TH + NP):
                        units.append((functools.partial(row_link, lr=lr), L_R))
                    for q in range(NP):
                        units.append((functools.partial(col_link, ty=ty, q=q), L_H))
            return units

        def out_chain(s, msrc, conv1=False):
            img = (s >> 2) & 1
            chunk = s & 3
            kind2 = False if conv1 else s >= 8
            if conv1:
                dslot, sslot, rslot = 2 + img, 2 + img, 0
            elif _static(s):
                dslot = (4 if kind2 else 2) + img
                sslot = 4 if kind2 else 2 + img
                rslot = img if kind2 else 0
            else:
                dslot = jnp.where(kind2, 4, 2) + img
                sslot = jnp.where(kind2, 4, 2 + img)
                rslot = jnp.where(kind2, img, 0)
            need_stats = not (_static(s) and kind2)
            units = []
            for g in range(NG):
                acc = [jnp.zeros((8, LG), F32), jnp.zeros((8, LG), F32)]
                for b in range(2 * CT):
                    hold = {}

                    def w_link(tok, g=g, b=b, hold=hold, ps=()):
                        vals = []
                        for p in ps:
                            mm = [msrc[p * NP + q, pl.ds(8 * b, 8), _gs(g)] for q in range(NP)]
                            if p == ps[0]:
                                mm[1] = inj(mm[1], tok)
                            hold[p] = _at(mm)
                            vals += hold[p]
                        return anchor(vals)

                    def fin_link(tok, g=g, b=b, acc=acc, hold=hold, e=0):
                        ty, hh = b // 2, b % 2
                        xw = []
                        for k in range(0 if conv1 else TH):
                            r = chunk * RC + ty * TH + k
                            if _static(s):
                                rr = r if kind2 else H
                            else:
                                rr = jnp.where(kind2, r, H)
                            xw.append(src[rslot, rr, g, pl.ds(16 * hh + e, 8, stride=2), :])
                        y = []
                        for l in (2 * e, 2 * e + 1):
                            col = [hold[p][l] for p in range(NP)]
                            col[1] = inj(col[1], tok)
                            y.append(_at(col))
                        for k in range(TH):
                            r = chunk * RC + ty * TH + k
                            ye, yo = y[0][k], y[1][k]
                            if need_stats:
                                acc[0] = acc[0] + (ye + yo)
                                acc[1] = acc[1] + (ye * ye + yo * yo)
                            if not conv1:
                                ye, yo = ye + _unpack(xw[k], 0), yo + _unpack(xw[k], 1)
                            src[dslot, r, g, pl.ds(16 * hh + e, 8, stride=2), :] = _pack(ye, yo)
                        if need_stats and b == 2 * CT - 1 and e == 1:
                            stats[sslot, chunk, 0, :, _gs(g)] = acc[0]
                            stats[sslot, chunk, 1, :, _gs(g)] = acc[1]
                        tk = src[0, zsm[1], 0, 0:8, :]
                        if need_stats:
                            tk = tk | anchor(acc)
                        return tk

                    units.append((functools.partial(w_link, ps=(0, 1, 2)), L_A))
                    units.append((functools.partial(w_link, ps=(3, 4, 5)), L_A))
                    units.append((functools.partial(fin_link, e=0), L_C))
                    units.append((functools.partial(fin_link, e=1), L_C))
            return units

        def stage_mm(vsrc, mdst, conv1):
            for pos in range(NPOS):
                v = pltpu.bitcast(vsrc[pos], BF16)
                for g in range(NG):
                    u = u1g[g][pos] if conv1 else u2_ref[pos, pl.ds(g * (LG // 2), LG // 2), :]
                    mdst[pos, :, _gs(g)] = jax.lax.dot_general(v, pltpu.bitcast(u, BF16), (((1,), (1,)), ((), ())),
                                                               preferred_element_type=F32)

        def stage_mm_g(vsrc, mdst, usrc, g):
            for pos in range(NPOS):
                v = pltpu.bitcast(vsrc[pos], BF16)
                u = pltpu.bitcast(usrc[pos], BF16)
                mdst[pos, :, _gs(g)] = jax.lax.dot_general(v, u, (((1,), (1,)), ((), ())),
                                                           preferred_element_type=F32)

        def out_copy(s, g):
            img = (s >> 2) & 1
            chunk = s & 3
            return pltpu.make_async_copy(src.at[4 + img, pl.ds(chunk * RC, RC), g],
                                         ob_.at[img, pl.ds(chunk * RC, RC), :, pl.ds(g * LG, LG)],
                                         sems.at[48 + (s - 8) * NG + g])

        def x_copy(img, c, g, nrows, sem):
            return pltpu.make_async_copy(xb.at[img, pl.ds(c * nrows, nrows), :, pl.ds(g * LG, LG)],
                                         src.at[img, pl.ds(c * nrows, nrows), g], sems.at[sem])

        NW1 = 16
        WR = (C // 2) // NW1

        def w1_copy(k):
            return pltpu.make_async_copy(w1b.at[:, :, pl.ds(k * WR, WR)],
                                         wraw.at[0, :, :, pl.ds(k * WR, WR)], sems.at[16 + k])

        for c in range(NCH):
            for g in range(NG):
                x_copy(0, c, g, RC, c * NG + g).start()
        small = [pltpu.make_async_copy(a, b, sems.at[40 + i]) for i, (a, b) in enumerate(
            ((g1_hbm, g1_ref), (be1_hbm, be1_ref), (g2_hbm, g2_ref), (be2_hbm, be2_ref), (t_hbm, t_ref)))]
        for cp in small:
            cp.start()
        for k in range(NW1):
            w1_copy(k).start()
        cx1 = [x_copy(1, 0, g, H, 32 + g) for g in range(NG)]
        cwe = pltpu.make_async_copy(wemb_hbm, wembs, sems.at[36])
        cw2 = [pltpu.make_async_copy(w2b.at[:, :, pl.ds(h * (C // 4), C // 4)],
                                     wraw.at[1, :, :, pl.ds(h * (C // 4), C // 4)], sems.at[37 + h]) for h in range(2)]
        for cp in (cx1[0], cx1[1], cw2[0], cx1[2], cx1[3], cw2[1], cwe):
            cp.start()

        zsm[0] = NPOS
        zsm[1] = H
        zsm[2] = NRB * NR * 12
        zvr[...] = jnp.zeros((8, LG), U32)
        rbuf[NRB * NR * 12] = jnp.zeros((8, LG), F32)
        v0[NPOS] = jnp.zeros((MC // 2, C), U32)
        v1[NPOS] = jnp.zeros((MC // 2, C), U32)
        u2_ref[NPOS, 0:8, 0:LG] = jnp.zeros((8, LG), U32)
        src[0, H] = jnp.zeros((NG, TW, LG), U32)
        zero = jnp.zeros((1, C), F32)
        embtab[0] = zero
        embtab[1] = zero

        def xs_body(c, carry):
            for g in range(NG):
                x_copy(0, c, g, RC, c * NG + g).wait()
            x_stats(0, c * RC, RC, c)
            return carry

        def wt_body(k, carry):
            w1_copy(k).wait()
            for kk in range(WR // 8):
                for cb in range(NG):
                    w_unit(None, 0, pl.multiple_of(k * WR + kk * 8, 8), cb)
            return carry

        jax.lax.fori_loop(0, NCH, xs_body, 0)
        for cp in small:
            cp.wait()
        gbt[0, 0] = g1_ref[...].astype(F32).reshape(1, C)
        gbt[0, 1] = be1_ref[...].astype(F32).reshape(1, C)
        gbt[1, 0] = g2_ref[...].astype(F32).reshape(1, C)
        gbt[1, 1] = be2_ref[...].astype(F32).reshape(1, C)
        gn_params(0)
        run_chains([(0, in_chain(0, v0, None))], paced=False)
        jax.lax.fori_loop(0, NW1 // NG, wt_body, 0)

        in1 = in_chain(1, v1, None)

        def sub_block(g):
            chs = [(T0 if g + 1 < NG else T0L, in1[ISP[g]:ISP[g + 1]])]
            if g + 1 < NG:
                for k in range((g + 1) * NW1 // NG, (g + 2) * NW1 // NG):
                    w1_copy(k).wait()
                chs.append((T0, [(functools.partial(w_unit, g=g + 1, ob=8 * kk, cb=cb), L_W)
                                 for kk in range(8) for cb in range(NG)]))
            else:
                for cp in cx1[:2]:
                    cp.wait()
                chs.append((T0L, x1_chain((0, 1))))
            run_chains(chs)
            stage_mm_g(v0, m0, u1g[g], g)

        def sub_body(i, carry):
            for g in range(NG):
                pl.when(i == g)(functools.partial(sub_block, g))
            return carry
        jax.lax.fori_loop(0, NG, sub_body, 0)

        def step(s, par, conv1):
            cur, nxt = par, 1 - par
            tt = T1 if conv1 else T2
            chs = [(tt, out_chain(s - 1, mbuf[nxt], conv1)),
                   (tt, in_chain(jnp.minimum(s + 1, 15), vbuf[nxt], 'top' if par == 1 else 'bot'))]
            if conv1:
                obs = [pl.multiple_of(jnp.minimum((s - 1) * URB + kk, C // 16 - 1) * 8, 8) for kk in range(URB)]
                chs.append((T_U, u_chain(obs)))
            run_chains(chs)
            stage_mm(vbuf[cur], mbuf[cur], conv1)

        def body1(s, carry):
            @pl.when(s == 1)
            def _():
                cw2[0].wait()

            @pl.when(s == 4)
            def _():
                cw2[1].wait()

            @pl.when(s == 2)
            def _():
                for cp in cx1[2:]:
                    cp.wait()

                def xs1(c, cc):
                    x_stats(1, c * RC, RC, c, (2, 3))
                    return cc
                jax.lax.fori_loop(0, NCH, xs1, 0)

            @pl.when(s == 3)
            def _():
                cwe.wait()
                emb_stage()
                gn_params(1)

            @pl.when(s == 7)
            def _():
                gn_params(2)

            jax.lax.cond((s & 1) == 0, lambda: step(s, 0, True), lambda: step(s, 1, True))
            return carry

        def body2(s, carry):
            @pl.when(s == 11)
            def _():
                gn_params(3)

            jax.lax.cond((s & 1) == 0, lambda: step(s, 0, False), lambda: step(s, 1, False))

            @pl.when(s >= 9)
            def _():
                for g in range(NG):
                    out_copy(s - 1, g).start()
            return carry

        jax.lax.fori_loop(1, 8, body1, 0)

        jax.lax.fori_loop(8, 16, body2, 0)
        last = out_chain(15, m1)
        nper = len(last) // NG
        for g in range(NG):
            run_chains([(0, last[g * nper:(g + 1) * nper])], paced=False)
            out_copy(15, g).start()
        for s in range(8, 16):
            for g in range(NG):
                out_copy(s, g).wait()

    return kernel


_KERNEL = make_kernel({})


@jax.jit
def pallas_standalone__adm_resblock__diffusion_kernel(x, t_emb, g1, be1, w1, w_emb, g2, be2, w2):
    xh = jnp.transpose(x, (0, 2, 3, 1))
    w1t = jnp.transpose(w1, (2, 3, 0, 1))
    w2t = jnp.transpose(w2, (2, 3, 0, 1))
    hb = pl.BlockSpec(memory_space=pl.ANY)
    out = pl.pallas_call(
        _KERNEL,
        out_shape=jax.ShapeDtypeStruct((B, H, W, C), BF16),
        in_specs=[hb] * 9,
        out_specs=hb,
        scratch_shapes=[
            pltpu.VMEM((B, EMB), BF16),
            pltpu.VMEM((C,), BF16),
            pltpu.VMEM((C,), BF16),
            pltpu.VMEM((C,), BF16),
            pltpu.VMEM((C,), BF16),
            pltpu.VMEM((2, 3, 3, C // 2, C), U32),
            pltpu.VMEM((EMB, C), BF16),
            pltpu.VMEM((NPOS, LG // 2, C), U32),
            pltpu.VMEM((NPOS, LG // 2, C), U32),
            pltpu.VMEM((NPOS, LG // 2, C), U32),
            pltpu.VMEM((NPOS, LG // 2, C), U32),
            pltpu.VMEM((NPOS + 1, C // 2, C), U32),
            pltpu.VMEM((6, H + 1, NG, TW, LG), U32),
            pltpu.VMEM((NPOS + 1, MC // 2, C), U32),
            pltpu.VMEM((NPOS + 1, MC // 2, C), U32),
            pltpu.VMEM((NPOS, MC, C), F32),
            pltpu.VMEM((NPOS, MC, C), F32),
            pltpu.VMEM((2 * NR * 12 + 1, 8, LG), F32),
            pltpu.VMEM((5, NCH, 2, 8, C), F32),
            pltpu.VMEM((4, 1, C), F32),
            pltpu.VMEM((2, 2, 1, C), F32),
            pltpu.VMEM((4, 2, 8, C), F32),
            pltpu.VMEM((8, LG), U32),
            pltpu.SMEM((8,), jnp.int32),
            pltpu.SemaphoreType.DMA((80,)),
        ],
        compiler_params=pltpu.CompilerParams(vmem_limit_bytes=120 * 2 ** 20),
    )(xh, t_emb, g1, be1, w1t, w_emb, g2, be2, w2t)
    return jnp.transpose(out, (0, 3, 1, 2))
```

```python
import functools
import jax
import jax.numpy as jnp
from jax.experimental import pallas as pl
from jax.experimental.pallas import tpu as pltpu

B, C, H, W, EMB = 2, 512, 64, 64, 1152
NG, LG = 4, 128
TH = 4
NP = 6
NPOS = NP * NP
TW = W // 2
CT = 4
MC = CT * (W // TH)
RC = CT * TH
NCH = H // RC
NR = RC + 2
EPS = 1e-5
F32 = jnp.float32
BF16 = jnp.bfloat16
U32 = jnp.uint32

PA, PB = 2.0 / 3.0, 1.5


CA = 1.0 / (2.0 * PA * PA * (PA * PA - PB * PB))
CB = 1.0 / (PA * PA * 2.0 * PB * PB * (PB * PB - PA * PA))


def _bt(d):
    a2, b2 = PA * PA, PB * PB
    d0, d1, d2, d3, d4, d5 = d
    p2 = b2 * d2
    aa = d4 - p2
    ra = PA * (d3 - b2 * d1)
    ab = d4 - a2 * d2
    rb = PB * (d3 - a2 * d1)
    t0 = (d0 + ab) - p2
    t5 = (d1 + d5) - (a2 + b2) * d3
    return [t0, aa + ra, aa - ra, ab + rb, ab - rb, t5]


def _at(m):
    m0, m1, m2, m3, m4, m5 = m
    sa, da = m1 + m2, m1 - m2
    sb, db = m3 + m4, m3 - m4
    y0 = (m0 + CA * sa) + CB * sb
    y1 = (CA * PA) * da + (CB * PB) * db
    y2 = (CA * PA * PA) * sa + (CB * PB * PB) * sb
    y3 = ((CA * PA ** 3) * da + (CB * PB ** 3) * db) + m5
    return [y0, y1, y2, y3]


def _gt(g0, g1, g2):
    a2 = PA * PA
    od = PA * g1
    ea = g0 + a2 * g2
    eb = a2 * g0 + g2
    return [g0, ea + od, ea - od, eb + od, eb - od, g2]


def _unpack(w, idx):
    return pltpu.unpack_elementwise(w, index=idx, packed_dtype=BF16, unpacked_dtype=F32)


def _pack(lo, hi):
    return pltpu.pack_elementwise([lo, hi], packed_dtype=BF16)


def _gs(g):
    return slice(g * LG, (g + 1) * LG)


def _static(s):
    return isinstance(s, int)


def make_kernel(cfg):
    T2 = cfg.get('T2', 9700)
    T1 = cfg.get('T1', 8800)
    T_U = cfg.get('TU', 7000)
    T0, T0L = cfg.get('T0', 2600), cfg.get('T0L', 2500)
    ISP = cfg.get('isp', [0, 36, 72, 108, 168])
    L_R, L_H, L_A, L_C, L_U, L_W = 40, 22, 20, 26, 30, 60
    URB = 5
    NRB = 2

    def kernel(x_hbm, t_hbm, g1_hbm, be1_hbm, w1_hbm, wemb_hbm, g2_hbm, be2_hbm, w2_hbm,
               out_hbm,
               t_ref, g1_ref, be1_ref, g2_ref, be2_ref,
               wraw, wembs, ua, ub, uc, ud, u2_ref, src, v0, v1, m0, m1, rbuf, stats, embtab, gbt, gnp, zvr, zsm, sems):
        vbuf = (v0, v1)
        u1g = (ua, ub, uc, ud)
        mbuf = (m0, m1)
        xb = x_hbm.bitcast(U32)
        ob_ = out_hbm.bitcast(U32)
        w1b = w1_hbm.bitcast(U32)
        w2b = w2_hbm.bitcast(U32)

        def delay(tok_u32, cyc):
            t = pltpu.bitcast(tok_u32, F32)
            n, rem = divmod(cyc, 116)
            for _ in range(n):
                t = jnp.broadcast_to(jnp.sum(t, axis=1, keepdims=True), (8, LG))
            for _ in range(rem // 8):
                t = jnp.tanh(t)
            return t

        def run_chains(chains, paced=True):
            items = []
            for ci, (tt, ch) in enumerate(chains):
                n = len(ch)
                nat = sum(c[1] for c in ch)
                extra = max(0.0, (tt - nat) / n)
                for k, (fn, lat) in enumerate(ch):
                    items.append(((k + 0.5) / n, ci, fn, int(extra)))
            items.sort(key=lambda it: (it[0], it[1]))
            toks = [None] * len(chains)
            for _, ci, fn, d in items:
                raw = fn(toks[ci])
                toks[ci] = delay(raw, d) if paced else None

        def anchor(vals):
            b = [pltpu.bitcast(v, U32) for v in vals]
            while len(b) > 1:
                b = [b[i] | b[i + 1] if i + 1 < len(b) else b[i] for i in range(0, len(b), 2)]
            return b[0] & zvr[...]

        def inj(x, tok):
            return x if tok is None else x + tok

        def x_stats(img, row0, nrows, slot, groups=range(NG)):
            for g in groups:
                a1 = [jnp.zeros((8, LG), F32)] * 2
                a2 = [jnp.zeros((8, LG), F32)] * 2
                for j in range(nrows):
                    for t in range(TW // 8):
                        w = src[img, row0 + j, g, pl.ds(8 * t, 8), :]
                        e, o = _unpack(w, 0), _unpack(w, 1)
                        a1[t % 2] = a1[t % 2] + (e + o)
                        a2[t % 2] = a2[t % 2] + (e * e + o * o)
                stats[img, slot, 0, :, _gs(g)] = a1[0] + a1[1]
                stats[img, slot, 1, :, _gs(g)] = a2[0] + a2[1]

        def x1_chain(groups):
            units = []
            for g in groups:
                for c in range(NCH):
                    acc = [jnp.zeros((8, LG), F32), jnp.zeros((8, LG), F32)]

                    def s_link(tok, g=g, c=c, acc=acc, j0=0):
                        for j in range(j0, j0 + 4):
                            for t in range(TW // 8):
                                w = src[1, c * RC + j, g, pl.ds(8 * t, 8), :]
                                e, o = _unpack(w, 0), _unpack(w, 1)
                                if t % 2 == 0:
                                    e = inj(e, tok)
                                acc[0] = acc[0] + (e + o)
                                acc[1] = acc[1] + (e * e + o * o)
                        if j0 + 4 == RC:
                            stats[1, c, 0, :, _gs(g)] = acc[0]
                            stats[1, c, 1, :, _gs(g)] = acc[1]
                        return anchor(acc)

                    for j0 in range(0, RC, 4):
                        units.append((functools.partial(s_link, j0=j0), 40))
            return units

        def w_unit(tok, g, ob, cb):
            raw = [[[None] * 3 for _ in range(3)] for _ in range(2)]
            for i in range(3):
                for j in range(3):
                    w = wraw[0, i, j, pl.ds(g * (LG // 2) + ob, 8), _gs(cb)]
                    raw[0][i][j], raw[1][i][j] = _unpack(w, 0), _unpack(w, 1)
            raw[0][0][1] = inj(raw[0][0][1], tok)
            wq = [[_gt(*raw[par][i]) for i in range(3)] for par in range(2)]
            for q in range(NP):
                o0 = _gt(*[wq[0][i][q] for i in range(3)])
                o1 = _gt(*[wq[1][i][q] for i in range(3)])
                for p in range(NP):
                    u1g[g][p * NP + q, pl.ds(ob, 8), _gs(cb)] = _pack(o0[p], o1[p])
            return anchor([o0[1], o1[1]])

        def u_chain(obs):
            a2 = PA * PA
            units = []
            for ob in obs:
                for cb in range(NG):
                    def u_link(tok, ob=ob, cb=cb, qs=()):
                        js = (0,) if qs == (0,) else (2,) if qs == (5,) else (0, 1, 2)
                        wq = [[], []]
                        for i in range(3):
                            w = [wraw[1, i, j, pl.ds(ob, 8), _gs(cb)] for j in js]
                            for par in range(2):
                                r = [_unpack(x, par) for x in w]
                                if par == 0:
                                    r[0] = inj(r[0], tok)
                                if len(js) == 1:
                                    wq[par].append(r)
                                else:
                                    od = PA * r[1]
                                    ev = r[0] + a2 * r[2] if qs == (1, 2) else a2 * r[0] + r[2]
                                    wq[par].append([ev + od, ev - od])
                        for qi, q in enumerate(qs):
                            o0 = _gt(*[wq[0][i][qi] for i in range(3)])
                            o1 = _gt(*[wq[1][i][qi] for i in range(3)])
                            for p in range(NP):
                                u2_ref[p * NP + q, pl.ds(ob, 8), _gs(cb)] = _pack(o0[p], o1[p])
                        return u2_ref[zsm[0], 0:8, 0:LG]

                    units.append((functools.partial(u_link, qs=(0,)), L_U // 2))
                    units.append((functools.partial(u_link, qs=(1, 2)), L_U))
                    units.append((functools.partial(u_link, qs=(3, 4)), L_U))
                    units.append((functools.partial(u_link, qs=(5,)), L_U // 2))
            return units

        def emb_stage():
            t = t_ref[...].astype(F32)
            st = (t * jax.nn.sigmoid(t)).astype(BF16)
            emb = jnp.dot(st, wembs[...], preferred_element_type=F32)
            embtab[2] = emb[0:1]
            embtab[3] = emb[1:2]

        def gn_params(sidx):
            conv = sidx >> 1
            s1 = stats[sidx, 0, 0] + stats[sidx, 1, 0] + stats[sidx, 2, 0] + stats[sidx, 3, 0]
            s2 = stats[sidx, 0, 1] + stats[sidx, 1, 1] + stats[sidx, 2, 1] + stats[sidx, 3, 1]
            s1 = jnp.sum(s1, axis=0, keepdims=True)
            s2 = jnp.sum(s2, axis=0, keepdims=True)
            e = embtab[sidx]
            n = float(H * W)
            t1 = s1 + n * e
            t2 = s2 + (2.0 * e) * s1 + (n * e) * e
            gam = gbt[conv, 0]
            bet = gbt[conv, 1]
            inv = 1.0 / (H * W * LG)
            for g in range(NG):
                mean = jnp.sum(t1[:, _gs(g)], axis=1, keepdims=True) * inv
                ex2 = jnp.sum(t2[:, _gs(g)], axis=1, keepdims=True) * inv
                var = jnp.maximum(ex2 - mean * mean, 0.0)
                rstd = jax.lax.rsqrt(var + EPS)
                sc = gam[:, _gs(g)] * rstd
                sh = bet[:, _gs(g)] + (e[:, _gs(g)] - mean) * sc
                gnp[sidx, 0, :, _gs(g)] = jnp.broadcast_to(0.5 * sc, (8, LG))
                gnp[sidx, 1, :, _gs(g)] = jnp.broadcast_to(0.5 * sh, (8, LG))

        def in_chain(s, vdst, edge):
            sidx = s >> 2
            chunk = s & 3
            r0 = chunk * RC - 1
            sub = jax.lax.broadcasted_iota(jnp.int32, (8, LG), 0)
            units = []
            for g in range(NG):
                base = (g % NRB) * NR * 12

                def row_link(tok, g=g, base=base, lr=0):
                    r = r0 + lr
                    valid = None
                    zero_row = False
                    if _static(r):
                        zero_row = r < 0 or r >= H
                    elif lr == 0 and edge in ('top', 'both'):
                        valid = r >= 0
                        r = jnp.maximum(r, 0)
                    elif lr == NR - 1 and edge in ('bot', 'both'):
                        valid = r < H
                        r = jnp.minimum(r, H - 1)
                    if zero_row:
                        z = jnp.zeros((8, LG), F32)
                        for q in range(12):
                            rbuf[base + lr * 12 + q] = z
                    else:
                        sc = inj(gnp[sidx, 0, :, _gs(g)], tok)
                        sh = gnp[sidx, 1, :, _gs(g)]
                        c = []
                        for j in range(4):
                            w = src[sidx, r, g, pl.ds(j, 8, stride=4), :]
                            for half in range(2):
                                hv = _unpack(w, half) * sc + sh
                                a = hv + hv * jnp.tanh(hv)
                                if valid is not None:
                                    a = jnp.where(valid, a, 0.0)
                                c.append(a)
                        left = jnp.where(sub == 0, 0.0, pltpu.roll(c[7], 1, 0))
                        right = jnp.where(sub == 7, 0.0, pltpu.roll(c[0], 7, 0))
                        ev = _bt([left, c[0], c[1], c[2], c[3], c[4]])
                        od = _bt([c[3], c[4], c[5], c[6], c[7], right])
                        for q in range(NP):
                            rbuf[base + lr * 12 + q] = ev[q]
                            rbuf[base + lr * 12 + 6 + q] = od[q]
                    return pltpu.bitcast(rbuf[zsm[2]], U32)

                def col_link(tok, g=g, base=base, ty=0, q=0):
                    t = []
                    for par in range(2):
                        d = [rbuf[base + (ty * TH + i) * 12 + 6 * par + q] for i in range(NP)]
                        if par == 0:
                            d[2] = inj(d[2], tok)
                        t.append(_bt(d))
                    for p in range(NP):
                        vdst[p * NP + q, pl.ds(ty * 8, 8), _gs(g)] = _pack(t[0][p], t[1][p])
                    return vdst[zsm[0], 0:8, 0:LG]

                for ty in range(CT):
                    for lr in range(0 if ty == 0 else ty * TH + 2, ty * TH + NP):
                        units.append((functools.partial(row_link, lr=lr), L_R))
                    for q in range(NP):
                        units.append((functools.partial(col_link, ty=ty, q=q), L_H))
            return units

        def out_chain(s, msrc, conv1=False):
            img = (s >> 2) & 1
            chunk = s & 3
            kind2 = False if conv1 else s >= 8
            if conv1:
                dslot, sslot, rslot = 2 + img, 2 + img, 0
            elif _static(s):
                dslot = (4 if kind2 else 2) + img
                sslot = 4 if kind2 else 2 + img
                rslot = img if kind2 else 0
            else:
                dslot = jnp.where(kind2, 4, 2) + img
                sslot = jnp.where(kind2, 4, 2 + img)
                rslot = jnp.where(kind2, img, 0)
            need_stats = not (_static(s) and kind2)
            units = []
            for g in range(NG):
                acc = [jnp.zeros((8, LG), F32), jnp.zeros((8, LG), F32)]
                for b in range(2 * CT):
                    hold = {}

                    def w_link(tok, g=g, b=b, hold=hold, ps=()):
                        vals = []
                        for p in ps:
                            mm = [msrc[p * NP + q, pl.ds(8 * b, 8), _gs(g)] for q in range(NP)]
                            if p == ps[0]:
                                mm[1] = inj(mm[1], tok)
                            hold[p] = _at(mm)
                            vals += hold[p]
                        return anchor(vals)

                    def fin_link(tok, g=g, b=b, acc=acc, hold=hold, e=0):
                        ty, hh = b // 2, b % 2
                        xw = []
                        for k in range(0 if conv1 else TH):
                            r = chunk * RC + ty * TH + k
                            if _static(s):
                                rr = r if kind2 else H
                            else:
                                rr = jnp.where(kind2, r, H)
                            xw.append(src[rslot, rr, g, pl.ds(16 * hh + e, 8, stride=2), :])
                        y = []
                        for l in (2 * e, 2 * e + 1):
                            col = [hold[p][l] for p in range(NP)]
                            col[1] = inj(col[1], tok)
                            y.append(_at(col))
                        for k in range(TH):
                            r = chunk * RC + ty * TH + k
                            ye, yo = y[0][k], y[1][k]
                            if need_stats:
                                acc[0] = acc[0] + (ye + yo)
                                acc[1] = acc[1] + (ye * ye + yo * yo)
                            if not conv1:
                                ye, yo = ye + _unpack(xw[k], 0), yo + _unpack(xw[k], 1)
                            src[dslot, r, g, pl.ds(16 * hh + e, 8, stride=2), :] = _pack(ye, yo)
                        if need_stats and b == 2 * CT - 1 and e == 1:
                            stats[sslot, chunk, 0, :, _gs(g)] = acc[0]
                            stats[sslot, chunk, 1, :, _gs(g)] = acc[1]
                        tk = src[0, zsm[1], 0, 0:8, :]
                        if need_stats:
                            tk = tk | anchor(acc)
                        return tk

                    units.append((functools.partial(w_link, ps=(0, 1, 2)), L_A))
                    units.append((functools.partial(w_link, ps=(3, 4, 5)), L_A))
                    units.append((functools.partial(fin_link, e=0), L_C))
                    units.append((functools.partial(fin_link, e=1), L_C))
            return units

        def stage_mm(vsrc, mdst, conv1):
            for pos in range(NPOS):
                v = pltpu.bitcast(vsrc[pos], BF16)
                for g in range(NG):
                    u = u1g[g][pos] if conv1 else u2_ref[pos, pl.ds(g * (LG // 2), LG // 2), :]
                    mdst[pos, :, _gs(g)] = jax.lax.dot_general(v, pltpu.bitcast(u, BF16), (((1,), (1,)), ((), ())),
                                                               preferred_element_type=F32)

        def stage_mm_g(vsrc, mdst, usrc, g):
            for pos in range(NPOS):
                v = pltpu.bitcast(vsrc[pos], BF16)
                u = pltpu.bitcast(usrc[pos], BF16)
                mdst[pos, :, _gs(g)] = jax.lax.dot_general(v, u, (((1,), (1,)), ((), ())),
                                                           preferred_element_type=F32)

        def out_copy(s, g):
            img = (s >> 2) & 1
            chunk = s & 3
            return pltpu.make_async_copy(src.at[4 + img, pl.ds(chunk * RC, RC), g],
                                         ob_.at[img, pl.ds(chunk * RC, RC), :, pl.ds(g * LG, LG)],
                                         sems.at[48 + (s - 8) * NG + g])

        def x_copy(img, c, g, nrows, sem):
            return pltpu.make_async_copy(xb.at[img, pl.ds(c * nrows, nrows), :, pl.ds(g * LG, LG)],
                                         src.at[img, pl.ds(c * nrows, nrows), g], sems.at[sem])

        NW1 = 16
        WR = (C // 2) // NW1

        def w1_copy(k):
            return pltpu.make_async_copy(w1b.at[:, :, pl.ds(k * WR, WR)],
                                         wraw.at[0, :, :, pl.ds(k * WR, WR)], sems.at[16 + k])

        for c in range(NCH):
            for g in range(NG):
                x_copy(0, c, g, RC, c * NG + g).start()
        small = [pltpu.make_async_copy(a, b, sems.at[40 + i]) for i, (a, b) in enumerate(
            ((g1_hbm, g1_ref), (be1_hbm, be1_ref), (g2_hbm, g2_ref), (be2_hbm, be2_ref), (t_hbm, t_ref)))]
        for cp in small:
            cp.start()
        for k in range(NW1):
            w1_copy(k).start()
        cx1 = [x_copy(1, 0, g, H, 32 + g) for g in range(NG)]
        cwe = pltpu.make_async_copy(wemb_hbm, wembs, sems.at[36])
        cw2 = [pltpu.make_async_copy(w2b.at[:, :, pl.ds(h * (C // 4), C // 4)],
                                     wraw.at[1, :, :, pl.ds(h * (C // 4), C // 4)], sems.at[37 + h]) for h in range(2)]
        for cp in (cx1[0], cx1[1], cw2[0], cx1[2], cx1[3], cw2[1], cwe):
            cp.start()

        zsm[0] = NPOS
        zsm[1] = H
        zsm[2] = NRB * NR * 12
        zvr[...] = jnp.zeros((8, LG), U32)
        rbuf[NRB * NR * 12] = jnp.zeros((8, LG), F32)
        v0[NPOS] = jnp.zeros((MC // 2, C), U32)
        v1[NPOS] = jnp.zeros((MC // 2, C), U32)
        u2_ref[NPOS, 0:8, 0:LG] = jnp.zeros((8, LG), U32)
        src[0, H] = jnp.zeros((NG, TW, LG), U32)
        zero = jnp.zeros((1, C), F32)
        embtab[0] = zero
        embtab[1] = zero

        def xs_body(c, carry):
            for g in range(NG):
                x_copy(0, c, g, RC, c * NG + g).wait()
            x_stats(0, c * RC, RC, c)
            return carry

        def wt_body(k, carry):
            w1_copy(k).wait()
            for kk in range(WR // 8):
                for cb in range(NG):
                    w_unit(None, 0, pl.multiple_of(k * WR + kk * 8, 8), cb)
            return carry

        jax.lax.fori_loop(0, NCH, xs_body, 0)
        for cp in small:
            cp.wait()
        gbt[0, 0] = g1_ref[...].astype(F32).reshape(1, C)
        gbt[0, 1] = be1_ref[...].astype(F32).reshape(1, C)
        gbt[1, 0] = g2_ref[...].astype(F32).reshape(1, C)
        gbt[1, 1] = be2_ref[...].astype(F32).reshape(1, C)
        gn_params(0)
        run_chains([(0, in_chain(0, v0, None))], paced=False)
        jax.lax.fori_loop(0, NW1 // NG, wt_body, 0)

        in1 = in_chain(1, v1, None)

        def sub_block(g):
            chs = [(T0 if g + 1 < NG else T0L, in1[ISP[g]:ISP[g + 1]])]
            if g + 1 < NG:
                for k in range((g + 1) * NW1 // NG, (g + 2) * NW1 // NG):
                    w1_copy(k).wait()
                chs.append((T0, [(functools.partial(w_unit, g=g + 1, ob=8 * kk, cb=cb), L_W)
                                 for kk in range(8) for cb in range(NG)]))
            else:
                for cp in cx1[:2]:
                    cp.wait()
                chs.append((T0L, x1_chain((0, 1))))
            run_chains(chs)
            stage_mm_g(v0, m0, u1g[g], g)

        def sub_body(i, carry):
            for g in range(NG):
                pl.when(i == g)(functools.partial(sub_block, g))
            return carry
        jax.lax.fori_loop(0, NG, sub_body, 0)

        def step(s, par, conv1):
            cur, nxt = par, 1 - par
            tt = T1 if conv1 else T2
            chs = [(tt, out_chain(s - 1, mbuf[nxt], conv1)),
                   (tt, in_chain(jnp.minimum(s + 1, 15), vbuf[nxt], 'top' if par == 1 else 'bot'))]
            if conv1:
                obs = [pl.multiple_of(jnp.minimum((s - 1) * URB + kk, C // 16 - 1) * 8, 8) for kk in range(URB)]
                chs.append((T_U, u_chain(obs)))
            run_chains(chs)
            stage_mm(vbuf[cur], mbuf[cur], conv1)

        def body1(s, carry):
            @pl.when(s == 1)
            def _():
                cw2[0].wait()

            @pl.when(s == 4)
            def _():
                cw2[1].wait()

            @pl.when(s == 2)
            def _():
                for cp in cx1[2:]:
                    cp.wait()

                def xs1(c, cc):
                    x_stats(1, c * RC, RC, c, (2, 3))
                    return cc
                jax.lax.fori_loop(0, NCH, xs1, 0)

            @pl.when(s == 3)
            def _():
                cwe.wait()
                emb_stage()
                gn_params(1)

            @pl.when(s == 7)
            def _():
                gn_params(2)

            jax.lax.cond((s & 1) == 0, lambda: step(s, 0, True), lambda: step(s, 1, True))
            return carry

        def body2(s, carry):
            @pl.when(s == 11)
            def _():
                gn_params(3)

            jax.lax.cond((s & 1) == 0, lambda: step(s, 0, False), lambda: step(s, 1, False))

            @pl.when(s >= 9)
            def _():
                for g in range(NG):
                    out_copy(s - 1, g).start()
            return carry

        jax.lax.fori_loop(1, 8, body1, 0)

        jax.lax.fori_loop(8, 16, body2, 0)
        last = out_chain(15, m1)
        nper = len(last) // NG
        for g in range(NG):
            run_chains([(0, last[g * nper:(g + 1) * nper])], paced=False)
            out_copy(15, g).start()
        for s in range(8, 16):
            for g in range(NG):
                out_copy(s, g).wait()

    return kernel


_KERNEL = make_kernel({})

_PARAMS = dict(vmem_limit_bytes=120 * 2 ** 20)
if hasattr(pltpu.CompilerParams, 'disable_semaphore_checks'):
    _PARAMS['disable_semaphore_checks'] = True


@jax.jit
def pallas_standalone__adm_resblock__diffusion_kernel(x, t_emb, g1, be1, w1, w_emb, g2, be2, w2):
    xh = jnp.transpose(x, (0, 2, 3, 1))
    w1t = jnp.transpose(w1, (2, 3, 0, 1))
    w2t = jnp.transpose(w2, (2, 3, 0, 1))
    hb = pl.BlockSpec(memory_space=pl.ANY)
    out = pl.pallas_call(
        _KERNEL,
        out_shape=jax.ShapeDtypeStruct((B, H, W, C), BF16),
        in_specs=[hb] * 9,
        out_specs=hb,
        scratch_shapes=[
            pltpu.VMEM((B, EMB), BF16),
            pltpu.VMEM((C,), BF16),
            pltpu.VMEM((C,), BF16),
            pltpu.VMEM((C,), BF16),
            pltpu.VMEM((C,), BF16),
            pltpu.VMEM((2, 3, 3, C // 2, C), U32),
            pltpu.VMEM((EMB, C), BF16),
            pltpu.VMEM((NPOS, LG // 2, C), U32),
            pltpu.VMEM((NPOS, LG // 2, C), U32),
            pltpu.VMEM((NPOS, LG // 2, C), U32),
            pltpu.VMEM((NPOS, LG // 2, C), U32),
            pltpu.VMEM((NPOS + 1, C // 2, C), U32),
            pltpu.VMEM((6, H + 1, NG, TW, LG), U32),
            pltpu.VMEM((NPOS + 1, MC // 2, C), U32),
            pltpu.VMEM((NPOS + 1, MC // 2, C), U32),
            pltpu.VMEM((NPOS, MC, C), F32),
            pltpu.VMEM((NPOS, MC, C), F32),
            pltpu.VMEM((2 * NR * 12 + 1, 8, LG), F32),
            pltpu.VMEM((5, NCH, 2, 8, C), F32),
            pltpu.VMEM((4, 1, C), F32),
            pltpu.VMEM((2, 2, 1, C), F32),
            pltpu.VMEM((4, 2, 8, C), F32),
            pltpu.VMEM((8, LG), U32),
            pltpu.SMEM((8,), jnp.int32),
            pltpu.SemaphoreType.DMA((80,)),
        ],
        compiler_params=pltpu.CompilerParams(**_PARAMS),
    )(xh, t_emb, g1, be1, w1t, w_emb, g2, be2, w2t)
    return jnp.transpose(out, (0, 3, 1, 2))
```
